```python
import jax
import jax.numpy as jnp

def _softmax(x, axis=-1):
    return jax.nn.softmax(x, axis=axis)

def _gelu(x):
    return jax.nn.gelu(x, approximate=True)

def _silu(x):
    return jax.nn.silu(x)

def _sigmoid(x):
    return jax.nn.sigmoid(x)

def _layernorm(x, axis=-1, eps=1e-05):
    m = jnp.mean(x, axis=axis, keepdims=True)
    v = jnp.var(x, axis=axis, keepdims=True)
    return (x - m) / jnp.sqrt(v + eps)

def _scatter_add(tgt, idx, src, axis=0):
    return tgt.at[idx].add(src)

def _segment_sum(src, seg, n):
    return jax.ops.segment_sum(src, seg, n)

class _Rng:

    def __init__(self, key):
        self._k = key

    def _next(self):
        self._k, sub = jax.random.split(self._k)
        return sub

    def normal(self, shape):
        return jax.random.normal(self._next(), shape, dtype=jnp.bfloat16)

    def randint(self, lo, hi, shape):
        return jax.random.randint(self._next(), shape, lo, hi, dtype=jnp.int32)

    def uniform(self, shape, lo=0.0, hi=1.0):
        return jax.random.uniform(self._next(), shape, jnp.bfloat16, lo, hi)

    def permutation(self, n):
        return jax.random.permutation(self._next(), n)
kernel_name = 'concat_heads__softmax_full_mha__memory_aug_recurrent_mem_tr__prompt'

def setup_inputs():
    _rng = _Rng(jax.random.key(int.from_bytes(__import__("os").urandom(4), "little")))
    _w = lambda a: (lambda t: t.astype(jnp.bfloat16) if jnp.issubdtype(t.dtype, jnp.floating) else t)(jnp.asarray(a))

    def _A_setup():
        B, S, D = (1, 2048, 1024)
        return {'x': _w((lambda *s: _rng.normal(s) * 0.05)(B, S, D)), 'wqkv': _w((lambda *s: _rng.normal(s) * 0.05)(D, 3 * D)), 'wo': _w((lambda *s: _rng.normal(s) * 0.05)(D, D))}
    _A_in = _A_setup()

    def _B_setup():
        B, S, Dm = (1, 2048, 1024)
        H, Dh = (32, 128)
        M, seg = (8, 32)
        seg = min(seg, S)
        S = S // seg * seg
        return {'x': _w((lambda *s: _rng.normal(s) * 0.05)(B, S, Dm)), 'mem0': _w((lambda *s: _rng.normal(s) * 0.05)(B, M, Dm)), 'Wq': _w((lambda *s: _rng.normal(s) * 0.05)(Dm, H, Dh) * Dm ** (-0.5)), 'Wk': _w((lambda *s: _rng.normal(s) * 0.05)(Dm, H, Dh) * Dm ** (-0.5)), 'Wv': _w((lambda *s: _rng.normal(s) * 0.05)(Dm, H, Dh) * Dm ** (-0.5)), 'Wo': _w((lambda *s: _rng.normal(s) * 0.05)(H, Dh, Dm) * (H * Dh) ** (-0.5)), 'seg_len': seg}
    _B_in = _B_setup()
    return {'A_x': _A_in['x'], 'A_wqkv': _A_in['wqkv'], 'A_wo': _A_in['wo'], 'B_x': _B_in['x'], 'B_mem0': _B_in['mem0'], 'B_Wq': _B_in['Wq'], 'B_Wk': _B_in['Wk'], 'B_Wv': _B_in['Wv'], 'B_Wo': _B_in['Wo'], 'B_seg_len': _B_in['seg_len']}

def reference(A_x, A_wqkv, A_wo, B_x, B_mem0, B_Wq, B_Wk, B_Wv, B_Wo, B_seg_len):

    def _A_ref(x, wqkv, wo):
        B, S, D = x.shape
        H = 32
        Dh = D // H
        qkv = (lambda x, *d: x.transpose(*d))((x @ wqkv).reshape(B, S, 3, H, Dh), 2, 0, 3, 1, 4)
        q, k, v = (qkv[0], qkv[1], qkv[2])
        scale = Dh ** (-0.5)
        scores = jnp.einsum('bhqd,bhkd->bhqk', q, k) * scale
        p = _softmax(scores, axis=-1)
        o = jnp.einsum('bhqk,bhkd->bhqd', p, v)
        return (lambda x, *d: x.transpose(*d))(o, 0, 2, 1, 3).reshape(B, S, D) @ wo

    def _B_ref(x, mem0, Wq, Wk, Wv, Wo, seg_len):
        B, S, Dm = x.shape
        H, Dh = (Wq.shape[1], Wq.shape[2])
        M = mem0.shape[1]
        scale = Dh ** (-0.5)
        n_seg = S // seg_len
        L = M + seg_len
        idx = jnp.arange(L)
        mask = (idx[:, None] < M) | (idx[:, None] >= idx[None, :])
        mem = mem0
        outs = []
        for s in range(n_seg):
            xs = x[:, s * seg_len:(s + 1) * seg_len, :].copy()
            h = jnp.concatenate([mem, xs], axis=1)
            q = jnp.einsum('btd,dhe->bhte', h, Wq)
            k = jnp.einsum('btd,dhe->bhte', h, Wk)
            v = jnp.einsum('btd,dhe->bhte', h, Wv)
            scores = jnp.einsum('bhqe,bhke->bhqk', q, k) * scale
            scores = jnp.where(mask[None, None], scores, -1000000000.0)
            p = _softmax(scores, axis=-1)
            o = jnp.einsum('bhqk,bhke->bhqe', p, v)
            o = jnp.einsum('bhte,hed->btd', o, Wo)
            mem = o[:, :M, :].copy()
            outs.append(o[:, M:, :])
        return jnp.concatenate(outs, axis=1)
    a = _A_ref(A_x, A_wqkv, A_wo)
    b = _B_ref(B_x, B_mem0, B_Wq, B_Wk, B_Wv, B_Wo, B_seg_len)
    return jnp.concatenate([a, b], axis=-1)
```

```python
import functools, math
import jax
import jax.numpy as jnp
from jax import lax
import jax.experimental.pallas as pl
import jax.experimental.pallas.tpu as pltpu

bf = jnp.bfloat16
f32 = jnp.float32
u32 = jnp.uint32
LOG2E = math.log2(math.e)

S = 2048
D = 1024
HA, DHA = 32, 32
HB, DHB = 32, 128
MEM, SEG = 8, 32
NSEG = S // SEG
L = MEM + SEG

TQ = 512
CK = 128
NQ = S // TQ
NC = S // CK
SK = 2
LAG_M, LAG_L, LAG_O = 2, 2, 3

NT = (((1,), (1,)), ((), ()))
TT = (((0,), (1,)), ((), ()))


def _as_bf(x):
    return pltpu.bitcast(x, bf)


def _as_u32(x):
    return pltpu.bitcast(x, u32)


def make_kernel(phases="123PB"):
  def kernel(xa_hbm, wqkv_hbm, woa_hbm, xb_hbm, mem0_hbm, wq_hbm, wk_hbm, wv_hbm, wob_hbm,
           out_hbm,
           xa, wqkv, woa, kk, qt, vt, oa, s0, s1, s2, s3,
           xb, wq, wk, wv, wob, f8, o8, outb, sems):
    s_refs = (s0, s1, s2, s3)

    def cp(src, dst, i):
        return pltpu.make_async_copy(src, dst, sems.at[i])

    c_xa = cp(xa_hbm, xa, 0)
    c_wqkv = cp(wqkv_hbm, wqkv, 1)
    c_xa.start()
    c_wqkv.start()
    c_xa.wait()
    c_wqkv.wait()
    c_woa = cp(woa_hbm, woa, 2)
    c_xb = cp(xb_hbm, xb.at[pl.ds(0, NSEG)], 3)
    c_wq = cp(wq_hbm, wq, 4)
    c_wk = cp(wk_hbm, wk, 5)
    c_wv = cp(wv_hbm, wv, 6)
    c_wob = [cp(wob_hbm.at[:, pl.ds(128 * c, 128)], wob.at[c], 8 + c) for c in range(8)]
    for c in [c_woa, c_xb, c_wq, c_wk, c_wv] + c_wob:
        c.start()

    if "1" in phases:
        qscale = (DHA ** -0.5) * LOG2E
        RC = 512
        def a1k(r, _):
            r0 = pl.multiple_of(r * RC, RC)
            y = jnp.dot(xa[pl.ds(r0, RC), :], wqkv[:, D:2 * D], preferred_element_type=f32)
            yu = _as_u32(y.astype(bf))
            for g in range(8):
                kk[g, pl.ds(pl.multiple_of(r * (RC // 2), RC // 2), RC // 2), :] = yu[:, 128 * g:128 * (g + 1)]
            return 0
        lax.fori_loop(0, S // RC, a1k, 0)
        CC = 256
        def a1qv(c, _):
            c0 = pl.multiple_of(c * CC, CC)
            y = lax.dot_general(wqkv[:, pl.ds(c0, CC)], xa[...], TT, preferred_element_type=f32)
            qt[pl.ds(pl.multiple_of(c * (CC // 2), CC // 2), CC // 2), :] = _as_u32((y * qscale).astype(bf))
            y = lax.dot_general(wqkv[:, pl.ds(2 * D + c0, CC)], xa[...], TT, preferred_element_type=f32)
            vt[pl.ds(pl.multiple_of(c * (CC // 2), CC // 2), CC // 2), :] = _as_u32(y.astype(bf))
            return 0
        lax.fori_loop(0, D // CC, a1qv, 0)

    if "2" in phases:
        def qpad(g, j, q0):
            q = _as_bf(qt[pl.ds(pl.multiple_of((4 * g + j) * 16, 16), 16), pl.ds(q0, TQ)])
            parts = []
            if j > 0:
                parts.append(jnp.zeros((32 * j, TQ), bf))
            parts.append(q)
            if j < 3:
                parts.append(jnp.zeros((32 * (3 - j), TQ), bf))
            return jnp.concatenate(parts, axis=0)

        def p1_chunk(g, w, c, sref, m8):
            k = _as_bf(kk[g, pl.ds(c * CK // 2, CK // 2), :])
            s = jnp.dot(k, w, preferred_element_type=f32)
            sref[pl.ds(c * CK, CK), :] = s
            mm = jnp.max(s.reshape(CK // 8, 8, TQ), axis=0)
            return mm if m8 is None else jnp.maximum(m8, mm)

        def p2_chunk(h, c, sref, m, l8, o):
            s = sref[pl.ds(c * CK, CK), :]
            p = jnp.exp2(s.reshape(CK // 8, 8, TQ) - m[None])
            ll = jnp.sum(p, axis=0)
            v = _as_bf(vt[pl.ds(pl.multiple_of(h * 16, 16), 16), pl.ds(c * CK, CK)])
            oo = jnp.dot(v, p.reshape(CK, TQ).astype(bf), preferred_element_type=f32)
            return (ll if l8 is None else l8 + ll), (oo if o is None else o + oo)

        def bmax(m8):
            return jnp.broadcast_to(jnp.max(m8, axis=0, keepdims=True), (8, TQ))

        w = qpad(0, 0, 0)
        m8 = None
        for c in range(NC):
            m8 = p1_chunk(0, w, c, s_refs[0], m8)
        m_init = bmax(m8)
        w = qpad(0, 1, 0)
        m8 = None
        for c in range(SK):
            m8 = p1_chunk(0, w, c, s_refs[1], m8)
        NI = 8 * NQ

        def a2(i, carry):
            m0, m8 = carry
            g = i // NQ
            q0 = pl.multiple_of((i % NQ) * TQ, TQ)
            inext = jnp.minimum(i + 1, NI - 1)
            gn = inext // NQ
            q0n = pl.multiple_of((inext % NQ) * TQ, TQ)
            never = jnp.full((8, TQ), i, jnp.int32) < 0
            hist = []
            ms = {0: m0}
            outs = []
            l8 = o = None
            for t in range(4 * NC):
                j, c = divmod(t, NC)
                j1, c1 = divmod(t + NC + SK, NC)
                g2, q2 = (g, q0) if j1 < 4 else (gn, q0n)
                if c1 == 0:
                    m8 = None
                w = qpad(g2, j1 % 4, q2)
                m8 = p1_chunk(g2, w, c1, s_refs[j1 % 4], m8)
                if c1 == NC - 1:
                    ms[j1] = bmax(m8)
                mt = ms[j]
                if len(hist) >= LAG_M:
                    mt = jnp.where(never, hist[-LAG_M][0], mt)
                if len(hist) >= LAG_L:
                    mt = jnp.where(never, hist[-LAG_L][1], mt)
                if len(hist) >= LAG_O:
                    oo = hist[-LAG_O][2]
                    for r in range(4):
                        mt = jnp.where(never, oo[8 * r:8 * r + 8], mt)
                if c == 0:
                    l8 = o = None
                l8, o = p2_chunk(4 * g + j, c, s_refs[j], mt, l8, o)
                hist.append((m8, l8, o))
                if c == NC - 1:
                    l = jnp.sum(l8, axis=0, keepdims=True)
                    outs.append(o * (1.0 / l))
            og = jnp.concatenate(outs, axis=0).T
            oa[g, pl.ds(pl.multiple_of((i % NQ) * (TQ // 2), TQ // 2), TQ // 2), :] = _as_u32(og.astype(bf))
            return ms[4], m8
        lax.fori_loop(0, NI, a2, (m_init, m8))

    c_woa.wait()
    if "3" in phases:
        RC = 512
        def a3(r, _):
            o = jnp.concatenate(
                [_as_bf(oa[g, pl.ds(pl.multiple_of(r * (RC // 2), RC // 2), RC // 2), :]) for g in range(8)], axis=1)
            y = jnp.dot(o, woa[...], preferred_element_type=f32)
            xa[pl.ds(pl.multiple_of(r * RC, RC), RC), :] = y.astype(bf)
            return 0
        lax.fori_loop(0, S // RC, a3, 0)
    c_outa = cp(xa, out_hbm.at[:, pl.ds(0, D)], 0)
    c_outa.start()

    c_xb.wait()
    c_wq.wait()
    c_wk.wait()
    c_wv.wait()
    for c in c_wob:
        c.wait()
    w32 = [w.bitcast(u32) for w in (wq, wk, wv)]
    wob32 = wob.bitcast(u32)
    if "P" in phases:
        def b0(b, _):
            for w in w32:
                res = []
                for j in range(16):
                    lo = w[b, pl.ds(j, 8, stride=32), :]
                    hi = w[b, pl.ds(16 + j, 8, stride=32), :]
                    res.append((lo & jnp.uint32(0xFFFF)) | (hi << 16))
                    res.append((lo >> 16) | (hi & jnp.uint32(0xFFFF0000)))
                w[b] = jnp.concatenate(res, axis=0)
            return 0
        lax.fori_loop(0, 64, b0, 0)

    def w_head(h):
        parts = []
        for w in w32:
            if isinstance(h, int):
                t = w[:, 8 * h:8 * h + 8, :]
            else:
                t = w[:, pl.ds(pl.multiple_of(8 * h, 8), 8), :]
            parts.append(_as_bf(t.reshape(512, 128)))
        return jnp.concatenate(parts, axis=1)

    def wo_rows(r0, n):
        return jnp.concatenate([_as_bf(wob32[c, pl.ds(r0 // 2, n // 2), :]) for c in range(8)], axis=1)

    if "B" in phases:
        bscale = (DHB ** -0.5) * LOG2E
        x8 = xb[0:NSEG, 0:8, :].reshape(NSEG * 8, D)
        def b1(h, _):
            y = jnp.dot(x8, w_head(h), preferred_element_type=f32)
            y = jnp.concatenate([y[:, :128] * bscale, y[:, 128:]], axis=1).astype(bf)
            f8[h] = y.reshape(NSEG, 8, 384)
            return 0
        lax.fori_loop(0, HB, b1, 0)

        c_mem = cp(mem0_hbm, xb.at[0, pl.ds(0, MEM), :], 7)
        c_mem.start()
        c_mem.wait()

        ri = lax.broadcasted_iota(jnp.int32, (L, L), 0)
        ci = lax.broadcasted_iota(jnp.int32, (L, L), 1)
        rpos = jnp.where(ri >= 32, ri - 32, ri)
        cpos = jnp.where(ci >= 32, ci - 32, ci)
        mask = (ri < MEM) | (ci < MEM) | (rpos >= cpos)
        neg = -1e9 * LOG2E

        def step(s, _):
            hs = xb[s]
            qkv = {}
            sc = {}
            os_ = {}
            def proj(h):
                y = jnp.dot(hs, w_head(h), preferred_element_type=f32)
                y = jnp.concatenate([y[:, :128] * bscale, y[:, 128:]], axis=1).astype(bf)
                qkv[h] = jnp.concatenate([y, f8[h, s]], axis=0)
            def score(h):
                y = qkv[h]
                t = lax.dot_general(y[:, 0:128], y[:, 128:256], NT, preferred_element_type=f32)
                t = jnp.where(mask, t, neg)
                m = jnp.max(t, axis=1, keepdims=True)
                p = jnp.exp2(t - m)
                l = jnp.sum(p, axis=1, keepdims=True)
                sc[h] = (p.astype(bf), l)
            def pv(h):
                p, l = sc[h]
                o = jnp.dot(p, qkv[h][:, 256:384], preferred_element_type=f32) * (1.0 / l)
                o = o.astype(bf)
                os_[h] = o[0:32]
                o8[s, :, 128 * h:128 * (h + 1)] = o[32:40]
            def wo(h0, h1):
                o = jnp.concatenate([os_[h] for h in range(h0, h1)], axis=1)
                return jnp.dot(o, wo_rows(128 * h0, 128 * (h1 - h0)), preferred_element_type=f32)
            for h in range(HB):
                proj(h)
                if h >= 1:
                    score(h - 1)
                if h >= 3:
                    pv(h - 3)
            acc = wo(0, 4)
            score(31)
            pv(29)
            acc = acc + wo(4, 8)
            pv(30)
            acc = acc + wo(8, 12)
            pv(31)
            acc = acc + wo(12, 32)
            y = acc.astype(bf)
            xb[s + 1, 0:8, :] = y[0:8]
            outb[s, 8:32, :] = y[8:32]
            return 0
        lax.fori_loop(0, NSEG, step, 0)

        RB = 16
        def b2(r, _):
            r0 = pl.multiple_of(r * RB, RB)
            o = o8[pl.ds(r0, RB)].reshape(RB * 8, HB * DHB)
            y = jnp.dot(o, wo_rows(0, HB * DHB), preferred_element_type=f32).astype(bf)
            outb[pl.ds(r0, RB), 0:8, :] = y.reshape(RB, 8, D)
            return 0
        lax.fori_loop(0, NSEG // RB, b2, 0)

    c_outa.wait()
    return_b = [cp(outb.at[s], out_hbm.at[pl.ds(32 * s, 32), pl.ds(D, D)], 1) for s in range(NSEG)]
    for c in return_b:
        c.start()
    for c in return_b:
        c.wait()
  return kernel


def build(phases="123PB"):
  @functools.partial(jax.jit, static_argnames=("B_seg_len",))
  def fn(A_x, A_wqkv, A_wo, B_x, B_mem0, B_Wq, B_Wk, B_Wv, B_Wo, B_seg_len):
    assert B_seg_len == SEG
    args = (
        A_x.reshape(S, D), A_wqkv, A_wo,
        B_x.reshape(NSEG, SEG, D), B_mem0.reshape(MEM, D),
        B_Wq.reshape(64, 512, 128), B_Wk.reshape(64, 512, 128), B_Wv.reshape(64, 512, 128),
        B_Wo.reshape(HB * DHB, D),
    )
    scratch = [
        pltpu.VMEM((S, D), bf),
        pltpu.VMEM((D, 3 * D), bf),
        pltpu.VMEM((D, D), bf),
        pltpu.VMEM((8, S // 2, 128), u32),
        pltpu.VMEM((D // 2, S), u32),
        pltpu.VMEM((D // 2, S), u32),
        pltpu.VMEM((8, S // 2, 128), u32),
        pltpu.VMEM((S, TQ), f32), pltpu.VMEM((S, TQ), f32), pltpu.VMEM((S, TQ), f32), pltpu.VMEM((S, TQ), f32),
        pltpu.VMEM((NSEG + 1, SEG, D), bf),
        pltpu.VMEM((64, 512, 128), bf), pltpu.VMEM((64, 512, 128), bf), pltpu.VMEM((64, 512, 128), bf),
        pltpu.VMEM((8, HB * DHB, 128), bf),
        pltpu.VMEM((HB, NSEG, 8, 384), bf),
        pltpu.VMEM((NSEG, 8, HB * DHB), bf),
        pltpu.VMEM((NSEG, SEG, D), bf),
        pltpu.SemaphoreType.DMA((16,)),
    ]
    out = pl.pallas_call(
        make_kernel(phases),
        out_shape=jax.ShapeDtypeStruct((S, 2 * D), bf),
        in_specs=[pl.BlockSpec(memory_space=pl.ANY)] * 9,
        out_specs=pl.BlockSpec(memory_space=pl.ANY),
        scratch_shapes=scratch,
        compiler_params=pltpu.CompilerParams(vmem_limit_bytes=126 * 1024 * 1024),
    )(*args)
    return out.reshape(1, S, 2 * D)
  return fn


pallas_concat_heads__softmax_full_mha__memory_aug_recurrent_mem_tr__prompt_kernel = build()
```

```python
import functools, math
import jax
import jax.numpy as jnp
from jax import lax
import jax.experimental.pallas as pl
import jax.experimental.pallas.tpu as pltpu

bf = jnp.bfloat16
f32 = jnp.float32
u32 = jnp.uint32
LOG2E = math.log2(math.e)

S = 2048
D = 1024
HA, DHA = 32, 32
HB, DHB = 32, 128
MEM, SEG = 8, 32
NSEG = S // SEG
L = MEM + SEG

TQ = 512
CK = 128
NQ = S // TQ
NC = S // CK
RC = 512
CC = 256
WP = 36
US = 4

NT = (((1,), (1,)), ((), ()))
TT = (((0,), (1,)), ((), ()))

CFG = dict(SK=2, LAG_M=2, LAG_L=2, LAG_O=3, SLAG=2, PVLAG=5, DYNL=0)


def _as_bf(x):
    return pltpu.bitcast(x, bf)


def _as_u32(x):
    return pltpu.bitcast(x, u32)


def make_kernel(phases, cfg):
  SK, LAG_M, LAG_L, LAG_O = cfg["SK"], cfg["LAG_M"], cfg["LAG_L"], cfg["LAG_O"]
  SLAG, PVLAG = cfg["SLAG"], cfg["PVLAG"]

  def kernel(xa_hbm, wqkv_hbm, woa_hbm, xb_hbm, mem0_hbm, wq_hbm, wk_hbm, wv_hbm, wob_hbm,
             out_hbm,
             xa, wqkv, woa, kk, qt, vt, oa, s0, s1, s2, s3,
             xb, m0v, wq, wk, wv, wob, outv, sems):
    s_refs = (s0, s1, s2, s3)

    def cp(src, dst, i):
        return pltpu.make_async_copy(src, dst, sems.at[i])

    c_wka = cp(wqkv_hbm.at[:, pl.ds(D, D)], wqkv.at[:, pl.ds(D, D)], 1)
    c_xa = [cp(xa_hbm.at[pl.ds(RC * r, RC)], xa.at[pl.ds(RC * r, RC)], 2 + r) for r in range(S // RC)]
    c_wqa = cp(wqkv_hbm.at[:, pl.ds(0, D)], wqkv.at[:, pl.ds(0, D)], 6)
    c_wva = cp(wqkv_hbm.at[:, pl.ds(2 * D, D)], wqkv.at[:, pl.ds(2 * D, D)], 7)
    c_wb = [cp(src.at[:, t], dst.at[:, pl.ds(2 * WP * t, 64), :], 8 + 8 * i + t)
            for i, (src, dst) in enumerate(((wq_hbm, wq), (wk_hbm, wk), (wv_hbm, wv))) for t in range(8)]
    c_late = [cp(wob_hbm.at[:, pl.ds(128 * c, 128)], wob.at[c], 32 + c) for c in range(8)]
    c_late += [cp(woa_hbm.at[:, pl.ds(128 * c, 128)], woa.at[c], 40 + c) for c in range(8)]
    c_late += [
        cp(xb_hbm, xb, 48),
        cp(mem0_hbm, m0v, 49),
    ]
    c_wka.start()
    c_xa[0].start()
    c_wka.wait()
    c_xa[0].wait()
    for c in c_xa[1:] + [c_wqa, c_wva]:
        c.start()

    qscale = (DHA ** -0.5) * LOG2E
    for r in range(S // RC):
        if r > 0:
            c_xa[r].wait()
        if "1" in phases:
            y = jnp.dot(xa[pl.ds(r * RC, RC), :], wqkv[:, D:2 * D], preferred_element_type=f32)
            yu = _as_u32(y.astype(bf))
            for g in range(8):
                kk[g, pl.ds(r * (RC // 2), RC // 2), :] = yu[:, 128 * g:128 * (g + 1)]
    c_wqa.wait()
    c_wva.wait()
    for c in c_wb + c_late:
        c.start()

    if "1" in phases:
        def a1qv(c, _):
            c0 = pl.multiple_of(c * CC, CC)
            y = lax.dot_general(wqkv[:, pl.ds(c0, CC)], xa[...], TT, preferred_element_type=f32)
            qt[pl.ds(pl.multiple_of(c * (CC // 2), CC // 2), CC // 2), :] = _as_u32((y * qscale).astype(bf))
            y = lax.dot_general(wqkv[:, pl.ds(2 * D + c0, CC)], xa[...], TT, preferred_element_type=f32)
            vt[pl.ds(pl.multiple_of(c * (CC // 2), CC // 2), CC // 2), :] = _as_u32(y.astype(bf))
            return 0
        lax.fori_loop(0, D // CC, a1qv, 0)

    for c in c_wb:
        c.wait()
    w32 = [w.bitcast(u32) for w in (wq, wk, wv)]

    def relayout(w, b):
        res = []
        for j in range(16):
            lo = w[b, pl.ds(j, 8, stride=WP), :]
            hi = w[b, pl.ds(16 + j, 8, stride=WP), :]
            res.append((lo & jnp.uint32(0xFFFF)) | (hi << 16))
            res.append((lo >> 16) | (hi & jnp.uint32(0xFFFF0000)))
        w[b, 0:256, :] = jnp.concatenate(res, axis=0)

    if "2" in phases:
        def qpad(g, j, q0):
            q = _as_bf(qt[pl.ds(pl.multiple_of((4 * g + j) * 16, 16), 16), pl.ds(q0, TQ)])
            parts = []
            if j > 0:
                parts.append(jnp.zeros((32 * j, TQ), bf))
            parts.append(q)
            if j < 3:
                parts.append(jnp.zeros((32 * (3 - j), TQ), bf))
            return jnp.concatenate(parts, axis=0)

        def p1_chunk(g, w, c, sref, m8):
            k = _as_bf(kk[g, pl.ds(c * CK // 2, CK // 2), :])
            s = jnp.dot(k, w, preferred_element_type=f32)
            sref[pl.ds(c * CK, CK), :] = s
            mm = jnp.max(s.reshape(CK // 8, 8, TQ), axis=0)
            return mm if m8 is None else jnp.maximum(m8, mm)

        def p2_chunk(h, c, sref, m, l8, o, z):
            s = sref[pl.ds(pl.multiple_of(z + c * CK, 8), CK), :]
            p = jnp.exp2(s.reshape(CK // 8, 8, TQ) - m[None])
            ll = jnp.sum(p, axis=0)
            v = _as_bf(vt[pl.ds(pl.multiple_of(h * 16, 16), 16), pl.ds(c * CK, CK)])
            oo = jnp.dot(v, p.reshape(CK, TQ).astype(bf), preferred_element_type=f32)
            return (ll if l8 is None else l8 + ll), (oo if o is None else o + oo)

        def bmax(m8):
            return jnp.broadcast_to(jnp.max(m8, axis=0, keepdims=True), (8, TQ))

        w = qpad(0, 0, 0)
        m8 = None
        for c in range(NC):
            m8 = p1_chunk(0, w, c, s_refs[0], m8)
        m_init = bmax(m8)
        w = qpad(0, 1, 0)
        m8 = None
        for c in range(SK):
            m8 = p1_chunk(0, w, c, s_refs[1], m8)
        NI = 8 * NQ

        def a2(i, carry):
            m0, m8 = carry
            g = i // NQ
            q0 = pl.multiple_of((i % NQ) * TQ, TQ)
            inext = jnp.minimum(i + 1, NI - 1)
            gn = inext // NQ
            q0n = pl.multiple_of((inext % NQ) * TQ, TQ)
            never = jnp.full((8, TQ), i, jnp.int32) < 0
            z = (i // 4096) * 8 if cfg["DYNL"] else 0
            hist = []
            ms = {0: m0}
            outs = []
            l8 = o = None
            for t in range(4 * NC):
                j, c = divmod(t, NC)
                j1, c1 = divmod(t + NC + SK, NC)
                g2, q2 = (g, q0) if j1 < 4 else (gn, q0n)
                if "P" in phases and t % 10 == 3 and t // 10 < 6:
                    relayout(w32[(t // 10) % 3], 2 * i + (t // 30))
                if c1 == 0:
                    m8 = None
                w = qpad(g2, j1 % 4, q2)
                m8 = p1_chunk(g2, w, c1, s_refs[j1 % 4], m8)
                if c1 == NC - 1:
                    ms[j1] = bmax(m8)
                mt = ms[j]
                if len(hist) >= LAG_M:
                    mt = jnp.where(never, hist[-LAG_M][0], mt)
                if len(hist) >= LAG_L:
                    mt = jnp.where(never, hist[-LAG_L][1], mt)
                if len(hist) >= LAG_O:
                    oo = hist[-LAG_O][2]
                    for r in range(4):
                        mt = jnp.where(never, oo[8 * r:8 * r + 8], mt)
                if c == 0:
                    l8 = o = None
                l8, o = p2_chunk(4 * g + j, c, s_refs[j], mt, l8, o, z)
                hist.append((m8, l8, o))
                if c == NC - 1:
                    l = jnp.sum(l8, axis=0, keepdims=True)
                    outs.append(o * (1.0 / l))
            og = jnp.concatenate(outs, axis=0).T
            oa[g, pl.ds(pl.multiple_of((i % NQ) * (TQ // 2), TQ // 2), TQ // 2), :] = _as_u32(og.astype(bf))
            return ms[4], m8
        lax.fori_loop(0, NI, a2, (m_init, m8))

    for c in c_late:
        c.wait()
    wob32 = wob.bitcast(u32)
    woa32 = woa.bitcast(u32)

    def w_head(h):
        return jnp.concatenate([_as_bf(w[:, 8 * h:8 * h + 8, :].reshape(512, 128)) for w in w32], axis=1)

    def wo_rows(r0, n):
        return jnp.concatenate([_as_bf(wob32[c, pl.ds(r0 // 2, n // 2), :]) for c in range(8)], axis=1)

    def out_copy(i):
        return cp(outv.at[pl.ds(i * US, US)], out_hbm.at[pl.ds(i * US, US)], 0)

    bscale = (DHB ** -0.5) * LOG2E
    ri = lax.broadcasted_iota(jnp.int32, (L, L), 0)
    ci = lax.broadcasted_iota(jnp.int32, (L, L), 1)
    rpos = jnp.where(ri >= 32, ri - 32, ri)
    cpos = jnp.where(ci >= 32, ci - 32, ci)
    mask = (ri < MEM) | (ci < MEM) | (rpos >= cpos)
    neg = -1e9 * LOG2E

    def bloop(i, mem):
        first8 = {}
        o8 = {}
        for u in range(US):
            s = i * US + u
            if "3" in phases:
                o = jnp.concatenate(
                    [_as_bf(oa[g, pl.ds(pl.multiple_of(s * 16, 16), 16), :]) for g in range(8)], axis=1)
                wa = jnp.concatenate([_as_bf(woa32[c]) for c in range(8)], axis=1)
                outv[s, :, 0:D] = jnp.dot(o, wa, preferred_element_type=f32).astype(bf)
            if "B" not in phases:
                continue
            parts = [mem, xb[s, MEM:SEG, :]]
            if u == 0:
                parts.append(xb[pl.ds(i * US, US), 0:MEM, :].reshape(US * MEM, D))
            hs = jnp.concatenate(parts, axis=0)
            qkv = {}
            sc = {}
            os_ = {}

            def proj(h):
                y = jnp.dot(hs, w_head(h), preferred_element_type=f32)
                y = jnp.concatenate([y[:, :128] * bscale, y[:, 128:]], axis=1)
                if u == 0:
                    first8[h] = y
                    qkv[h] = y[0:L].astype(bf)
                else:
                    qkv[h] = jnp.concatenate([y, first8[h][32 + 8 * u:40 + 8 * u]], axis=0).astype(bf)

            def score(h):
                y = qkv[h]
                t = lax.dot_general(y[:, 0:128], y[:, 128:256], NT, preferred_element_type=f32)
                t = jnp.where(mask, t, neg)
                m = jnp.max(t, axis=1, keepdims=True)
                p = jnp.exp2(t - m)
                l = jnp.sum(p, axis=1, keepdims=True)
                sc[h] = (p * (1.0 / l)).astype(bf)

            def pv(h):
                o = jnp.dot(sc[h], qkv[h][:, 256:384], preferred_element_type=f32)
                o8[u, h] = o[32:40]
                if u == US - 1:
                    os_[h] = jnp.concatenate([o[0:32]] + [o8[v, h] for v in range(US)], axis=0).astype(bf)
                else:
                    os_[h] = o[0:32].astype(bf)

            def wo(h0, h1):
                o = jnp.concatenate([os_[h] for h in range(h0, h1)], axis=1)
                return jnp.dot(o, wo_rows(128 * h0, 128 * (h1 - h0)), preferred_element_type=f32)

            acc = None
            for h in range(HB + PVLAG):
                if h < HB:
                    proj(h)
                else:
                    k = h - HB
                    part = wo(3 * k, 3 * k + 3)
                    acc = part if acc is None else acc + part
                if SLAG <= h < HB + SLAG:
                    score(h - SLAG)
                if h >= PVLAG:
                    pv(h - PVLAG)
            acc = acc + wo(3 * PVLAG, HB)
            y = acc.astype(bf)
            mem = y[0:8]
            outv[s, 8:32, D:2 * D] = y[8:32]
            if u == US - 1:
                outv[pl.ds(i * US, US), 0:8, D:2 * D] = acc[32:64].reshape(US, 8, D).astype(bf)
        out_copy(i).start()
        return mem
    lax.fori_loop(0, NSEG // US, bloop, m0v[...])

    for i in range(NSEG // US):
        out_copy(i).wait()
  return kernel


def build(phases="123PB", **kw):
  cfg = dict(CFG)
  cfg.update(kw)

  @functools.partial(jax.jit, static_argnames=("B_seg_len",))
  def fn(A_x, A_wqkv, A_wo, B_x, B_mem0, B_Wq, B_Wk, B_Wv, B_Wo, B_seg_len):
    assert B_seg_len == SEG
    args = (
        A_x.reshape(S, D), A_wqkv, A_wo,
        B_x.reshape(NSEG, SEG, D), B_mem0.reshape(MEM, D),
        B_Wq.reshape(64, 8, 64, 128), B_Wk.reshape(64, 8, 64, 128), B_Wv.reshape(64, 8, 64, 128),
        B_Wo.reshape(HB * DHB, D),
    )
    scratch = [
        pltpu.VMEM((S, D), bf),
        pltpu.VMEM((D, 3 * D), bf),
        pltpu.VMEM((8, D, 128), bf),
        pltpu.VMEM((8, S // 2, 128), u32),
        pltpu.VMEM((D // 2, S), u32),
        pltpu.VMEM((D // 2, S), u32),
        pltpu.VMEM((8, S // 2, 128), u32),
        pltpu.VMEM((S, TQ), f32), pltpu.VMEM((S, TQ), f32), pltpu.VMEM((S, TQ), f32), pltpu.VMEM((S, TQ), f32),
        pltpu.VMEM((NSEG, SEG, D), bf),
        pltpu.VMEM((MEM, D), bf),
        pltpu.VMEM((64, 16 * WP, 128), bf), pltpu.VMEM((64, 16 * WP, 128), bf), pltpu.VMEM((64, 16 * WP, 128), bf),
        pltpu.VMEM((8, HB * DHB, 128), bf),
        pltpu.VMEM((NSEG, SEG, 2 * D), bf),
        pltpu.SemaphoreType.DMA((50,)),
    ]
    out = pl.pallas_call(
        make_kernel(phases, cfg),
        out_shape=jax.ShapeDtypeStruct((NSEG, SEG, 2 * D), bf),
        in_specs=[pl.BlockSpec(memory_space=pl.ANY)] * 9,
        out_specs=pl.BlockSpec(memory_space=pl.ANY),
        scratch_shapes=scratch,
        compiler_params=pltpu.CompilerParams(vmem_limit_bytes=126 * 1024 * 1024),
    )(*args)
    return out.reshape(1, S, 2 * D)
  return fn


pallas_concat_heads__softmax_full_mha__memory_aug_recurrent_mem_tr__prompt_kernel = build()
```

```python
import functools, math
import jax
import jax.numpy as jnp
from jax import lax
import jax.experimental.pallas as pl
import jax.experimental.pallas.tpu as pltpu

bf = jnp.bfloat16
f32 = jnp.float32
u32 = jnp.uint32
LOG2E = math.log2(math.e)

S = 2048
D = 1024
HA, DHA = 32, 32
HB, DHB = 32, 128
MEM, SEG = 8, 32
NSEG = S // SEG
L = MEM + SEG

TQ = 512
CK = 128
NQ = S // TQ
NC = S // CK
RC = 512
CC = 256
WP = 36
US = 4

NT = (((1,), (1,)), ((), ()))
TT = (((0,), (1,)), ((), ()))

CFG = dict(SK=2, LAG_M=2, LAG_L=2, LAG_O=3, SLAG=2, PVLAG=5, T0=8, BI=1)


def _as_bf(x):
    return pltpu.bitcast(x, bf)


def _as_u32(x):
    return pltpu.bitcast(x, u32)


def make_kernel(phases, cfg):
  SK, LAG_M, LAG_L, LAG_O = cfg["SK"], cfg["LAG_M"], cfg["LAG_L"], cfg["LAG_O"]
  SLAG, PVLAG = cfg["SLAG"], cfg["PVLAG"]

  def kernel(xa_hbm, wqkv_hbm, woa_hbm, xb_hbm, mem0_hbm, wq_hbm, wk_hbm, wv_hbm, wob_hbm,
             out_hbm,
             xa, wqkv, woa, kk, qt, vt, oa, s0, s1, s2, s3,
             xb, m0v, wq, wk, wv, wob, outv, cnt, sems):
    s_refs = (s0, s1, s2, s3)

    def cp(src, dst, i):
        return pltpu.make_async_copy(src, dst, sems.at[i])

    c_wka = cp(wqkv_hbm.at[:, pl.ds(D, D)], wqkv.at[:, pl.ds(D, D)], 1)
    c_xa = [cp(xa_hbm.at[pl.ds(RC * r, RC)], xa.at[pl.ds(RC * r, RC)], 2 + r) for r in range(S // RC)]
    c_wqa = cp(wqkv_hbm.at[:, pl.ds(0, D)], wqkv.at[:, pl.ds(0, D)], 6)
    c_wva = cp(wqkv_hbm.at[:, pl.ds(2 * D, D)], wqkv.at[:, pl.ds(2 * D, D)], 7)
    c_wb = [cp(src.at[:, t], dst.at[pl.ds(1, 64), pl.ds(2 * WP * t, 64), :], 8 + 8 * i + t)
            for i, (src, dst) in enumerate(((wq_hbm, wq), (wk_hbm, wk), (wv_hbm, wv))) for t in range(8)]
    c_late = [cp(wob_hbm.at[:, pl.ds(128 * c, 128)], wob.at[c], 32 + c) for c in range(8)]
    c_late += [cp(woa_hbm.at[:, pl.ds(128 * c, 128)], woa.at[c], 40 + c) for c in range(8)]
    c_late += [
        cp(xb_hbm, xb, 48),
        cp(mem0_hbm, m0v, 49),
    ]
    c_wka.start()
    c_xa[0].start()
    c_wka.wait()
    c_xa[0].wait()
    for c in c_xa[1:] + [c_wqa, c_wva]:
        c.start()

    qscale = (DHA ** -0.5) * LOG2E
    for r in range(S // RC):
        if r > 0:
            c_xa[r].wait()
        if "1" in phases:
            y = jnp.dot(xa[pl.ds(r * RC, RC), :], wqkv[:, D:2 * D], preferred_element_type=f32)
            yu = _as_u32(y.astype(bf))
            for g in range(8):
                kk[g, pl.ds(r * (RC // 2), RC // 2), :] = yu[:, 128 * g:128 * (g + 1)]
    c_wqa.wait()
    c_wva.wait()
    for c in c_wb + c_late:
        c.start()

    if "1" in phases:
        def a1qv(c, _):
            c0 = pl.multiple_of(c * CC, CC)
            y = lax.dot_general(wqkv[:, pl.ds(c0, CC)], xa[...], TT, preferred_element_type=f32)
            qt[pl.ds(pl.multiple_of(c * (CC // 2), CC // 2), CC // 2), :] = _as_u32((y * qscale).astype(bf))
            y = lax.dot_general(wqkv[:, pl.ds(2 * D + c0, CC)], xa[...], TT, preferred_element_type=f32)
            vt[pl.ds(pl.multiple_of(c * (CC // 2), CC // 2), CC // 2), :] = _as_u32(y.astype(bf))
            cnt[0] = c
            return 0
        lax.fori_loop(0, D // CC, a1qv, 0)

    for c in c_wb:
        c.wait()
    w32 = [w.bitcast(u32) for w in (wq, wk, wv)]

    def relayout(w, b, j, tie):
        lo = tie(w[b + 1, pl.ds(j, 8, stride=WP), :])
        hi = tie(w[b + 1, pl.ds(16 + j, 8, stride=WP), :])
        w[b, 16 * j:16 * j + 8, :] = (lo & jnp.uint32(0xFFFF)) | (hi << 16)
        w[b, 16 * j + 8:16 * j + 16, :] = (lo >> 16) | (hi & jnp.uint32(0xFFFF0000))

    if "2" in phases:
        def mul(x, n):
            return x * n if isinstance(x, int) else pl.multiple_of(x * n, n)

        def qpad(g, j, qi):
            q = _as_bf(qt[pl.ds(mul(4 * g + j, 16), 16), pl.ds(mul(qi, TQ), TQ)])
            parts = []
            if j > 0:
                parts.append(jnp.zeros((32 * j, TQ), bf))
            parts.append(q)
            if j < 3:
                parts.append(jnp.zeros((32 * (3 - j), TQ), bf))
            return jnp.concatenate(parts, axis=0)

        def p1_chunk(g, w, c, sref, m8):
            k = _as_bf(kk[g, pl.ds(c * CK // 2, CK // 2), :])
            s = jnp.dot(k, w, preferred_element_type=f32)
            sref[pl.ds(c * CK, CK), :] = s
            mm = jnp.max(s.reshape(CK // 8, 8, TQ), axis=0)
            return mm if m8 is None else jnp.maximum(m8, mm)

        def p2_chunk(h, c, sref, m, l8, o):
            s = sref[pl.ds(c * CK, CK), :]
            p = jnp.exp2(s.reshape(CK // 8, 8, TQ) - m[None])
            ll = jnp.sum(p, axis=0)
            v = _as_bf(vt[pl.ds(mul(h, 16), 16), pl.ds(c * CK, CK)])
            oo = jnp.dot(v, p.reshape(CK, TQ).astype(bf), preferred_element_type=f32)
            return (ll if l8 is None else l8 + ll), (oo if o is None else o + oo)

        def bmax(m8):
            return jnp.broadcast_to(jnp.max(m8, axis=0, keepdims=True), (8, TQ))

        NI = 8 * NQ
        UL = 4 * NC
        LEAD = NC + SK

        def stream(t_lo, t_hi, ib, state, flag, p1_end, rl):
            mcur, m8, l8, o = state
            never = jnp.full((8, TQ), flag, jnp.int32) < 0
            nev1 = jnp.full((8, 128), flag, jnp.int32) < 0
            gq = {}
            for dlt in range(0, (t_hi + LEAD) // UL + 1):
                gq[dlt] = ((ib + dlt) // NQ, (ib + dlt) % NQ)
            ms = {max(t_lo, 0) // NC: mcur}
            hist = []
            outs = []
            for t in range(t_lo, t_hi):
                if t + LEAD < p1_end:
                    u1, c1 = divmod(t + LEAD, NC)
                    g2, q2 = gq[u1 // 4]
                    if c1 == 0:
                        m8 = None
                    m8 = p1_chunk(g2, qpad(g2, u1 % 4, q2), c1, s_refs[u1 % 4], m8)
                    if c1 == NC - 1:
                        ms[u1] = bmax(m8)
                if t in rl:
                    anchor = _as_u32(m8[:, 0:128])
                    for wi, bi, ji in rl[t]:
                        relayout(w32[wi], bi, ji, lambda x: jnp.where(nev1, anchor, x))
                if t < 0:
                    continue
                u, c = divmod(t, NC)
                g, qi = gq[u // 4]
                mt = ms[u]
                if len(hist) >= LAG_M:
                    mt = jnp.where(never, hist[-LAG_M][0], mt)
                if len(hist) >= LAG_L:
                    mt = jnp.where(never, hist[-LAG_L][1], mt)
                if len(hist) >= LAG_O:
                    oo = hist[-LAG_O][2]
                    for r in range(4):
                        mt = jnp.where(never, oo[8 * r:8 * r + 8], mt)
                if c == 0:
                    l8 = o = None
                l8, o = p2_chunk(4 * g + u % 4, c, s_refs[u % 4], mt, l8, o)
                hist.append((m8, l8, o))
                if c == NC - 1:
                    l = jnp.sum(l8, axis=0, keepdims=True)
                    outs.append(o * (1.0 / l))
                    if u % 4 == 3:
                        og = jnp.concatenate(outs, axis=0).T
                        oa[g, pl.ds(mul(qi, TQ // 2), TQ // 2), :] = _as_u32(og.astype(bf))
                        outs = []
            return ms.get(t_hi // NC), m8, l8, o

        T0 = cfg["T0"]
        BI = cfg["BI"]
        NL = (NI - 1) // BI
        BIG = 1 << 30

        def rl_plan(t_lo, nblk, b0):
            plan = {}
            if "P" in phases:
                for n in range(48 * nblk):
                    plan.setdefault(t_lo + 2 + n // 3, []).append((n % 3, b0 + n // 48, (n // 3) % 16))
            return plan

        state = stream(-LEAD, T0, 0, (None, None, None, None), cnt[0], BIG, {})

        def a2(i, state):
            return stream(T0, T0 + BI * UL, i * BI, state, i, BIG, rl_plan(T0, 2 * BI, 2 * BI * i))
        state = lax.fori_loop(0, NL, a2, state)
        rem = NI - NL * BI
        stream(T0, rem * UL, NL * BI, state, cnt[0], rem * UL, rl_plan(T0, 2 * rem, 2 * BI * NL))

    for c in c_late:
        c.wait()
    wob32 = wob.bitcast(u32)
    woa32 = woa.bitcast(u32)

    def w_head(h):
        return jnp.concatenate([_as_bf(w[0:64, 8 * h:8 * h + 8, :].reshape(512, 128)) for w in w32], axis=1)

    def wo_rows(r0, n):
        return jnp.concatenate([_as_bf(wob32[c, pl.ds(r0 // 2, n // 2), :]) for c in range(8)], axis=1)

    def out_copy(i):
        return cp(outv.at[pl.ds(i * US, US)], out_hbm.at[pl.ds(i * US, US)], 0)

    bscale = (DHB ** -0.5) * LOG2E
    ri = lax.broadcasted_iota(jnp.int32, (L, L), 0)
    ci = lax.broadcasted_iota(jnp.int32, (L, L), 1)
    rpos = jnp.where(ri >= 32, ri - 32, ri)
    cpos = jnp.where(ci >= 32, ci - 32, ci)
    mask = (ri < MEM) | (ci < MEM) | (rpos >= cpos)
    neg = -1e9 * LOG2E

    def bloop(i, mem):
        first8 = {}
        o8 = {}
        for u in range(US):
            s = i * US + u
            if "3" in phases:
                o = jnp.concatenate(
                    [_as_bf(oa[g, pl.ds(pl.multiple_of(s * 16, 16), 16), :]) for g in range(8)], axis=1)
                wa = jnp.concatenate([_as_bf(woa32[c]) for c in range(8)], axis=1)
                outv[s, :, 0:D] = jnp.dot(o, wa, preferred_element_type=f32).astype(bf)
            if "B" not in phases:
                continue
            parts = [mem, xb[s, MEM:SEG, :]]
            if u == 0:
                parts.append(xb[pl.ds(i * US, US), 0:MEM, :].reshape(US * MEM, D))
            hs = jnp.concatenate(parts, axis=0)
            qkv = {}
            sc = {}
            os_ = {}

            def proj(h):
                y = jnp.dot(hs, w_head(h), preferred_element_type=f32)
                y = jnp.concatenate([y[:, :128] * bscale, y[:, 128:]], axis=1)
                if u == 0:
                    first8[h] = y
                    qkv[h] = y[0:L].astype(bf)
                else:
                    qkv[h] = jnp.concatenate([y, first8[h][32 + 8 * u:40 + 8 * u]], axis=0).astype(bf)

            def score(h):
                y = qkv[h]
                t = lax.dot_general(y[:, 0:128], y[:, 128:256], NT, preferred_element_type=f32)
                t = jnp.where(mask, t, neg)
                m = jnp.max(t, axis=1, keepdims=True)
                p = jnp.exp2(t - m)
                l = jnp.sum(p, axis=1, keepdims=True)
                sc[h] = (p * (1.0 / l)).astype(bf)

            def pv(h):
                o = jnp.dot(sc[h], qkv[h][:, 256:384], preferred_element_type=f32)
                o8[u, h] = o[32:40]
                if u == US - 1:
                    os_[h] = jnp.concatenate([o[0:32]] + [o8[v, h] for v in range(US)], axis=0).astype(bf)
                else:
                    os_[h] = o[0:32].astype(bf)

            def wo(h0, h1):
                o = jnp.concatenate([os_[h] for h in range(h0, h1)], axis=1)
                return jnp.dot(o, wo_rows(128 * h0, 128 * (h1 - h0)), preferred_element_type=f32)

            acc = None
            for h in range(HB + PVLAG):
                if h < HB:
                    proj(h)
                else:
                    k = h - HB
                    part = wo(3 * k, 3 * k + 3)
                    acc = part if acc is None else acc + part
                if SLAG <= h < HB + SLAG:
                    score(h - SLAG)
                if h >= PVLAG:
                    pv(h - PVLAG)
            acc = acc + wo(3 * PVLAG, HB)
            y = acc.astype(bf)
            mem = y[0:8]
            outv[s, 8:32, D:2 * D] = y[8:32]
            if u == US - 1:
                outv[pl.ds(i * US, US), 0:8, D:2 * D] = acc[32:64].reshape(US, 8, D).astype(bf)
        out_copy(i).start()
        return mem
    lax.fori_loop(0, NSEG // US, bloop, m0v[...])

    for i in range(NSEG // US):
        out_copy(i).wait()
  return kernel


def build(phases="123PB", **kw):
  cfg = dict(CFG)
  cfg.update(kw)

  @functools.partial(jax.jit, static_argnames=("B_seg_len",))
  def fn(A_x, A_wqkv, A_wo, B_x, B_mem0, B_Wq, B_Wk, B_Wv, B_Wo, B_seg_len):
    assert B_seg_len == SEG
    args = (
        A_x.reshape(S, D), A_wqkv, A_wo,
        B_x.reshape(NSEG, SEG, D), B_mem0.reshape(MEM, D),
        B_Wq.reshape(64, 8, 64, 128), B_Wk.reshape(64, 8, 64, 128), B_Wv.reshape(64, 8, 64, 128),
        B_Wo.reshape(HB * DHB, D),
    )
    scratch = [
        pltpu.VMEM((S, D), bf),
        pltpu.VMEM((D, 3 * D), bf),
        pltpu.VMEM((8, D, 128), bf),
        pltpu.VMEM((8, S // 2, 128), u32),
        pltpu.VMEM((D // 2, S), u32),
        pltpu.VMEM((D // 2, S), u32),
        pltpu.VMEM((8, S // 2, 128), u32),
        pltpu.VMEM((S, TQ), f32), pltpu.VMEM((S, TQ), f32), pltpu.VMEM((S, TQ), f32), pltpu.VMEM((S, TQ), f32),
        pltpu.VMEM((NSEG, SEG, D), bf),
        pltpu.VMEM((MEM, D), bf),
        pltpu.VMEM((65, 16 * WP, 128), bf), pltpu.VMEM((65, 16 * WP, 128), bf), pltpu.VMEM((65, 16 * WP, 128), bf),
        pltpu.VMEM((8, HB * DHB, 128), bf),
        pltpu.VMEM((NSEG, SEG, 2 * D), bf),
        pltpu.SMEM((1,), jnp.int32),
        pltpu.SemaphoreType.DMA((50,)),
    ]
    out = pl.pallas_call(
        make_kernel(phases, cfg),
        out_shape=jax.ShapeDtypeStruct((NSEG, SEG, 2 * D), bf),
        in_specs=[pl.BlockSpec(memory_space=pl.ANY)] * 9,
        out_specs=pl.BlockSpec(memory_space=pl.ANY),
        scratch_shapes=scratch,
        compiler_params=pltpu.CompilerParams(vmem_limit_bytes=126 * 1024 * 1024),
    )(*args)
    return out.reshape(1, S, 2 * D)
  return fn


pallas_concat_heads__softmax_full_mha__memory_aug_recurrent_mem_tr__prompt_kernel = build()
```

```python
import functools, math
import jax
import jax.numpy as jnp
from jax import lax
import jax.experimental.pallas as pl
import jax.experimental.pallas.tpu as pltpu

bf = jnp.bfloat16
f32 = jnp.float32
u32 = jnp.uint32
LOG2E = math.log2(math.e)

S = 2048
D = 1024
HA, DHA = 32, 32
HB, DHB = 32, 128
MEM, SEG = 8, 32
NSEG = S // SEG
L = MEM + SEG

TQ = 512
CK = 128
NQ = S // TQ
NC = S // CK
RC = 512
CC = 256
WP = 36
US = 4

NT = (((1,), (1,)), ((), ()))
TT = (((0,), (1,)), ((), ()))

CFG = dict(SK=2, LAG_M=2, LAG_L=2, LAG_O=3, SLAG=2, PVLAG=5, T0=8, BI=1, NF=10)


def _as_bf(x):
    return pltpu.bitcast(x, bf)


def _as_u32(x):
    return pltpu.bitcast(x, u32)


def make_kernel(phases, cfg):
  SK, LAG_M, LAG_L, LAG_O = cfg["SK"], cfg["LAG_M"], cfg["LAG_L"], cfg["LAG_O"]
  SLAG, PVLAG = cfg["SLAG"], cfg["PVLAG"]

  def kernel(xa_hbm, wqkv_hbm, woa_hbm, xb_hbm, mem0_hbm, wq_hbm, wk_hbm, wv_hbm, wob_hbm,
             out_hbm,
             xa, wqkv, woa, kk, qt, vt, oa, s0, s1, s2, s3,
             xb, m0v, wq, wk, wv, wob, outv, cnt, sems):
    s_refs = (s0, s1, s2, s3)

    def cp(src, dst, i):
        return pltpu.make_async_copy(src, dst, sems.at[i])

    xr = [(0, 256), (256, 512), (512, 1024), (1024, 1536), (1536, 2048)]
    wc = [(0, 256), (256, 512), (512, 1024)]
    c_xa = [cp(xa_hbm.at[pl.ds(lo, hi - lo)], xa.at[pl.ds(lo, hi - lo)], 1 + r) for r, (lo, hi) in enumerate(xr)]
    c_wka = [cp(wqkv_hbm.at[:, pl.ds(D + lo, hi - lo)], wqkv.at[:, pl.ds(D + lo, hi - lo)], 50 + r)
             for r, (lo, hi) in enumerate(wc)]
    c_wqa = cp(wqkv_hbm.at[:, pl.ds(0, D)], wqkv.at[:, pl.ds(0, D)], 6)
    c_wva = cp(wqkv_hbm.at[:, pl.ds(2 * D, D)], wqkv.at[:, pl.ds(2 * D, D)], 7)
    c_wb = [cp(src.at[:, t], dst.at[pl.ds(1, 64), pl.ds(2 * WP * t, 64), :], 8 + 8 * i + t)
            for i, (src, dst) in enumerate(((wq_hbm, wq), (wk_hbm, wk), (wv_hbm, wv))) for t in range(8)]
    c_late = [cp(wob_hbm.at[:, pl.ds(128 * c, 128)], wob.at[c], 32 + c) for c in range(8)]
    c_late += [cp(woa_hbm.at[:, pl.ds(128 * c, 128)], woa.at[c], 40 + c) for c in range(8)]
    c_late += [
        cp(xb_hbm, xb, 48),
        cp(mem0_hbm, m0v, 49),
    ]
    first = [c_xa[0], c_wka[0], c_wka[1], c_xa[1], c_wka[2], c_xa[2], c_xa[3], c_xa[4], c_wqa, c_wva]
    NF = cfg["NF"]
    for c in first[:NF]:
        c.start()

    qscale = (DHA ** -0.5) * LOG2E

    def kproj(r0, r1, c0, c1):
        if "1" in phases:
            y = jnp.dot(xa[r0:r1, :], wqkv[:, D + c0:D + c1], preferred_element_type=f32)
            yu = _as_u32(y.astype(bf))
            for g in range(c0 // 128, c1 // 128):
                kk[g, r0 // 2:r1 // 2, :] = yu[:, 128 * g - c0:128 * (g + 1) - c0]

    c_xa[0].wait()
    c_wka[0].wait()
    for c in first[NF:]:
        c.start()
    kproj(0, 256, 0, 256)
    c_wka[1].wait()
    kproj(0, 256, 256, 512)
    c_xa[1].wait()
    kproj(256, 512, 0, 512)
    c_wka[2].wait()
    kproj(0, 512, 512, 1024)
    c_xa[2].wait()
    kproj(512, 1024, 0, 1024)
    c_xa[3].wait()
    c_xa[4].wait()
    for c in c_wb:
        c.start()
    kproj(1024, 1536, 0, 1024)
    kproj(1536, 2048, 0, 1024)
    c_wqa.wait()
    c_wva.wait()

    if "1" in phases:
        def a1qv(c, _):
            c0 = pl.multiple_of(c * CC, CC)
            y = lax.dot_general(wqkv[:, pl.ds(c0, CC)], xa[...], TT, preferred_element_type=f32)
            qt[pl.ds(pl.multiple_of(c * (CC // 2), CC // 2), CC // 2), :] = _as_u32((y * qscale).astype(bf))
            y = lax.dot_general(wqkv[:, pl.ds(2 * D + c0, CC)], xa[...], TT, preferred_element_type=f32)
            vt[pl.ds(pl.multiple_of(c * (CC // 2), CC // 2), CC // 2), :] = _as_u32(y.astype(bf))
            cnt[0] = c
            return 0
        lax.fori_loop(0, D // CC, a1qv, 0)

    for c in c_wb:
        c.wait()
    for c in c_late:
        c.start()
    w32 = [w.bitcast(u32) for w in (wq, wk, wv)]

    def relayout(w, b, j, tie):
        lo = tie(w[b + 1, pl.ds(j, 8, stride=WP), :])
        hi = tie(w[b + 1, pl.ds(16 + j, 8, stride=WP), :])
        w[b, 16 * j:16 * j + 8, :] = (lo & jnp.uint32(0xFFFF)) | (hi << 16)
        w[b, 16 * j + 8:16 * j + 16, :] = (lo >> 16) | (hi & jnp.uint32(0xFFFF0000))

    if "2" in phases:
        def mul(x, n):
            return x * n if isinstance(x, int) else pl.multiple_of(x * n, n)

        def qpad(g, j, qi):
            q = _as_bf(qt[pl.ds(mul(4 * g + j, 16), 16), pl.ds(mul(qi, TQ), TQ)])
            parts = []
            if j > 0:
                parts.append(jnp.zeros((32 * j, TQ), bf))
            parts.append(q)
            if j < 3:
                parts.append(jnp.zeros((32 * (3 - j), TQ), bf))
            return jnp.concatenate(parts, axis=0)

        def p1_chunk(g, w, c, sref, m8):
            k = _as_bf(kk[g, pl.ds(c * CK // 2, CK // 2), :])
            s = jnp.dot(k, w, preferred_element_type=f32)
            sref[pl.ds(c * CK, CK), :] = s
            mm = jnp.max(s.reshape(CK // 8, 8, TQ), axis=0)
            return mm if m8 is None else jnp.maximum(m8, mm)

        def p2_chunk(h, c, sref, m, l8, o):
            s = sref[pl.ds(c * CK, CK), :]
            p = jnp.exp2(s.reshape(CK // 8, 8, TQ) - m[None])
            ll = jnp.sum(p, axis=0)
            v = _as_bf(vt[pl.ds(mul(h, 16), 16), pl.ds(c * CK, CK)])
            oo = jnp.dot(v, p.reshape(CK, TQ).astype(bf), preferred_element_type=f32)
            return (ll if l8 is None else l8 + ll), (oo if o is None else o + oo)

        def bmax(m8):
            return jnp.broadcast_to(jnp.max(m8, axis=0, keepdims=True), (8, TQ))

        NI = 8 * NQ
        UL = 4 * NC
        LEAD = NC + SK

        def stream(t_lo, t_hi, ib, state, flag, p1_end, rl):
            mcur, m8, l8, o = state
            never = jnp.full((8, TQ), flag, jnp.int32) < 0
            nev1 = jnp.full((8, 128), flag, jnp.int32) < 0
            gq = {}
            for dlt in range(0, (t_hi + LEAD) // UL + 1):
                gq[dlt] = ((ib + dlt) // NQ, (ib + dlt) % NQ)
            ms = {max(t_lo, 0) // NC: mcur}
            hist = []
            outs = []
            for t in range(t_lo, t_hi):
                if t + LEAD < p1_end:
                    u1, c1 = divmod(t + LEAD, NC)
                    g2, q2 = gq[u1 // 4]
                    if c1 == 0:
                        m8 = None
                    m8 = p1_chunk(g2, qpad(g2, u1 % 4, q2), c1, s_refs[u1 % 4], m8)
                    if c1 == NC - 1:
                        ms[u1] = bmax(m8)
                if t in rl:
                    anchor = _as_u32(m8[:, 0:128])
                    for wi, bi, ji in rl[t]:
                        relayout(w32[wi], bi, ji, lambda x: jnp.where(nev1, anchor, x))
                if t < 0:
                    continue
                u, c = divmod(t, NC)
                g, qi = gq[u // 4]
                mt = ms[u]
                if len(hist) >= LAG_M:
                    mt = jnp.where(never, hist[-LAG_M][0], mt)
                if len(hist) >= LAG_L:
                    mt = jnp.where(never, hist[-LAG_L][1], mt)
                if len(hist) >= LAG_O:
                    oo = hist[-LAG_O][2]
                    for r in range(4):
                        mt = jnp.where(never, oo[8 * r:8 * r + 8], mt)
                if c == 0:
                    l8 = o = None
                l8, o = p2_chunk(4 * g + u % 4, c, s_refs[u % 4], mt, l8, o)
                hist.append((m8, l8, o))
                if c == NC - 1:
                    l = jnp.sum(l8, axis=0, keepdims=True)
                    outs.append(o * (1.0 / l))
                    if u % 4 == 3:
                        og = jnp.concatenate(outs, axis=0).T
                        oa[g, pl.ds(mul(qi, TQ // 2), TQ // 2), :] = _as_u32(og.astype(bf))
                        outs = []
            return ms.get(t_hi // NC), m8, l8, o

        T0 = cfg["T0"]
        BI = cfg["BI"]
        NL = (NI - 1) // BI
        BIG = 1 << 30

        def rl_plan(t_lo, nblk, b0):
            plan = {}
            if "P" in phases:
                for n in range(48 * nblk):
                    plan.setdefault(t_lo + 2 + n // 3, []).append((n % 3, b0 + n // 48, (n // 3) % 16))
            return plan

        state = stream(-LEAD, T0, 0, (None, None, None, None), cnt[0], BIG, {})

        def a2(i, state):
            return stream(T0, T0 + BI * UL, i * BI, state, i, BIG, rl_plan(T0, 2 * BI, 2 * BI * i))
        state = lax.fori_loop(0, NL, a2, state)
        rem = NI - NL * BI
        stream(T0, rem * UL, NL * BI, state, cnt[0], rem * UL, rl_plan(T0, 2 * rem, 2 * BI * NL))

    for c in c_late:
        c.wait()
    wob32 = wob.bitcast(u32)
    woa32 = woa.bitcast(u32)

    def w_head(h):
        return jnp.concatenate([_as_bf(w[0:64, 8 * h:8 * h + 8, :].reshape(512, 128)) for w in w32], axis=1)

    def wo_rows(r0, n):
        return jnp.concatenate([_as_bf(wob32[c, pl.ds(r0 // 2, n // 2), :]) for c in range(8)], axis=1)

    def out_copy(i):
        return cp(outv.at[pl.ds(i * US, US)], out_hbm.at[pl.ds(i * US, US)], 0)

    bscale = (DHB ** -0.5) * LOG2E
    neg = -1e9 * LOG2E
    ri = lax.broadcasted_iota(jnp.int32, (SEG, L), 0)
    ci = lax.broadcasted_iota(jnp.int32, (SEG, L), 1)
    mask = (ri < MEM) | (ci < MEM) | (ci >= SEG) | (ri >= ci)
    G = US * MEM
    ri = lax.broadcasted_iota(jnp.int32, (G, 3 * G), 0)
    ci = lax.broadcasted_iota(jnp.int32, (G, 3 * G), 1)
    own8 = (ci % G) // MEM == ri // MEM
    vis8 = own8 & ((ci < G) | ((ci < 2 * G) & (ci % MEM <= ri % MEM)))
    fill8 = jnp.where(own8, neg, -jnp.inf).astype(f32)
    mult8 = jnp.where(ci >= 2 * G, float((SEG - MEM) // MEM), 1.0).astype(f32)

    def bloop(i, mem):
        first8 = {}
        kv8 = {}
        for u in range(US):
            s = i * US + u
            if "3" in phases:
                o = jnp.concatenate(
                    [_as_bf(oa[g, pl.ds(pl.multiple_of(s * 16, 16), 16), :]) for g in range(8)], axis=1)
                wa = jnp.concatenate([_as_bf(woa32[c]) for c in range(8)], axis=1)
                outv[s, :, 0:D] = jnp.dot(o, wa, preferred_element_type=f32).astype(bf)
            if "B" not in phases:
                continue
            parts = [mem, xb[s, MEM:SEG, :]]
            if u == 0:
                parts.append(xb[pl.ds(i * US, US), 0:MEM, :].reshape(US * MEM, D))
            hs = jnp.concatenate(parts, axis=0)
            qkv = {}
            sc = {}
            sc8 = {}
            os_ = {}

            def proj(h):
                y = jnp.dot(hs, w_head(h), preferred_element_type=f32)
                q = (y[:, 0:128] * bscale).astype(bf)
                if u == 0:
                    first8[h] = (q[SEG:], y[SEG:, 128:384])
                kv = jnp.concatenate([y[0:SEG, 128:384], first8[h][1][MEM * u:MEM * (u + 1)]], axis=0).astype(bf)
                qkv[h] = (q[0:SEG], kv)
                kv8[u, h] = (y[0:MEM, 128:384], y[8:16, 256:384] + y[16:24, 256:384] + y[24:32, 256:384])

            def score(h):
                q, kv = qkv[h]
                t = lax.dot_general(q, kv[:, 0:128], NT, preferred_element_type=f32)
                t = jnp.where(mask, t, neg)
                m = jnp.max(t, axis=1, keepdims=True)
                p = jnp.exp2(t - m)
                l = jnp.sum(p, axis=1, keepdims=True)
                sc[h] = (p * (1.0 / l)).astype(bf)
                if u == US - 1:
                    kv = jnp.concatenate([kv8[v, h][0] for v in range(US)] + [first8[h][1]], axis=0).astype(bf)
                    t = lax.dot_general(first8[h][0], kv[:, 0:128], NT, preferred_element_type=f32)
                    t = jnp.concatenate([t, jnp.zeros((G, G), f32)], axis=1)
                    t = jnp.where(vis8, t, fill8)
                    m = jnp.max(t, axis=1, keepdims=True)
                    p = jnp.exp2(t - m)
                    l = jnp.sum(p * mult8, axis=1, keepdims=True)
                    vx = jnp.concatenate([kv8[v, h][1] for v in range(US)], axis=0).astype(bf)
                    sc8[h] = ((p * (1.0 / l)).astype(bf), jnp.concatenate([kv[:, 128:256], vx], axis=0))

            def pv(h):
                o = jnp.dot(sc[h], qkv[h][1][:, 128:256], preferred_element_type=f32).astype(bf)
                if u == US - 1:
                    o8 = jnp.dot(sc8[h][0], sc8[h][1], preferred_element_type=f32).astype(bf)
                    o = jnp.concatenate([o, o8], axis=0)
                os_[h] = o

            def wo(h0, h1):
                o = jnp.concatenate([os_[h] for h in range(h0, h1)], axis=1)
                return jnp.dot(o, wo_rows(128 * h0, 128 * (h1 - h0)), preferred_element_type=f32)

            acc = None
            for h in range(HB + PVLAG):
                if h < HB:
                    proj(h)
                else:
                    k = h - HB
                    part = wo(3 * k, 3 * k + 3)
                    acc = part if acc is None else acc + part
                if SLAG <= h < HB + SLAG:
                    score(h - SLAG)
                if h >= PVLAG:
                    pv(h - PVLAG)
            acc = acc + wo(3 * PVLAG, HB)
            y = acc.astype(bf)
            mem = y[0:8]
            outv[s, 8:32, D:2 * D] = y[8:32]
            if u == US - 1:
                outv[pl.ds(i * US, US), 0:8, D:2 * D] = acc[32:64].reshape(US, 8, D).astype(bf)
        out_copy(i).start()
        return mem
    lax.fori_loop(0, NSEG // US, bloop, m0v[...])

    for i in range(NSEG // US):
        out_copy(i).wait()
  return kernel


def build(phases="123PB", **kw):
  cfg = dict(CFG)
  cfg.update(kw)

  @functools.partial(jax.jit, static_argnames=("B_seg_len",))
  def fn(A_x, A_wqkv, A_wo, B_x, B_mem0, B_Wq, B_Wk, B_Wv, B_Wo, B_seg_len):
    assert B_seg_len == SEG
    args = (
        A_x.reshape(S, D), A_wqkv, A_wo,
        B_x.reshape(NSEG, SEG, D), B_mem0.reshape(MEM, D),
        B_Wq.reshape(64, 8, 64, 128), B_Wk.reshape(64, 8, 64, 128), B_Wv.reshape(64, 8, 64, 128),
        B_Wo.reshape(HB * DHB, D),
    )
    scratch = [
        pltpu.VMEM((S, D), bf),
        pltpu.VMEM((D, 3 * D), bf),
        pltpu.VMEM((8, D, 128), bf),
        pltpu.VMEM((8, S // 2, 128), u32),
        pltpu.VMEM((D // 2, S), u32),
        pltpu.VMEM((D // 2, S), u32),
        pltpu.VMEM((8, S // 2, 128), u32),
        pltpu.VMEM((S, TQ), f32), pltpu.VMEM((S, TQ), f32), pltpu.VMEM((S, TQ), f32), pltpu.VMEM((S, TQ), f32),
        pltpu.VMEM((NSEG, SEG, D), bf),
        pltpu.VMEM((MEM, D), bf),
        pltpu.VMEM((65, 16 * WP, 128), bf), pltpu.VMEM((65, 16 * WP, 128), bf), pltpu.VMEM((65, 16 * WP, 128), bf),
        pltpu.VMEM((8, HB * DHB, 128), bf),
        pltpu.VMEM((NSEG, SEG, 2 * D), bf),
        pltpu.SMEM((1,), jnp.int32),
        pltpu.SemaphoreType.DMA((53,)),
    ]
    out = pl.pallas_call(
        make_kernel(phases, cfg),
        out_shape=jax.ShapeDtypeStruct((NSEG, SEG, 2 * D), bf),
        in_specs=[pl.BlockSpec(memory_space=pl.ANY)] * 9,
        out_specs=pl.BlockSpec(memory_space=pl.ANY),
        scratch_shapes=scratch,
        compiler_params=pltpu.CompilerParams(vmem_limit_bytes=126 * 1024 * 1024),
    )(*args)
    return out.reshape(1, S, 2 * D)
  return fn


pallas_concat_heads__softmax_full_mha__memory_aug_recurrent_mem_tr__prompt_kernel = build()
```

```python
import functools, math
import jax
import jax.numpy as jnp
from jax import lax
import jax.experimental.pallas as pl
import jax.experimental.pallas.tpu as pltpu

bf = jnp.bfloat16
f32 = jnp.float32
u32 = jnp.uint32
LOG2E = math.log2(math.e)

S = 2048
D = 1024
HA, DHA = 32, 32
HB, DHB = 32, 128
MEM, SEG = 8, 32
NSEG = S // SEG
L = MEM + SEG

TQ = 512
CK = 128
NQ = S // TQ
NC = S // CK
RC = 512
CC = 256
WP = 36
US = 4

NT = (((1,), (1,)), ((), ()))
TT = (((0,), (1,)), ((), ()))

CFG = dict(SK=2, LAG_M=2, LAG_L=2, LAG_O=3, SLAG=2, PVLAG=5, T0=8, BI=1, NF=10, STIE=1, SROW=0, KLAG=2, OROWS=1)


def _as_bf(x):
    return pltpu.bitcast(x, bf)


def _as_u32(x):
    return pltpu.bitcast(x, u32)


def make_kernel(phases, cfg):
  SK, LAG_M, LAG_L, LAG_O = cfg["SK"], cfg["LAG_M"], cfg["LAG_L"], cfg["LAG_O"]
  SLAG, PVLAG = cfg["SLAG"], cfg["PVLAG"]

  def kernel(xa_hbm, wqkv_hbm, woa_hbm, xb_hbm, mem0_hbm, wq_hbm, wk_hbm, wv_hbm, wob_hbm,
             out_hbm,
             xa, wqkv, woa, kk, qt, vt, oa, s0, s1, s2, s3,
             xb, m0v, wq, wk, wv, wob, outv, cnt, sems):
    s_refs = (s0, s1, s2, s3)

    def cp(src, dst, i):
        return pltpu.make_async_copy(src, dst, sems.at[i])

    xr = [(0, 256), (256, 512), (512, 1024), (1024, 1536), (1536, 2048)]
    wc = [(0, 256), (256, 512), (512, 1024)]
    c_xa = [cp(xa_hbm.at[pl.ds(lo, hi - lo)], xa.at[pl.ds(lo, hi - lo)], 1 + r) for r, (lo, hi) in enumerate(xr)]
    c_wka = [cp(wqkv_hbm.at[:, pl.ds(D + lo, hi - lo)], wqkv.at[:, pl.ds(D + lo, hi - lo)], 50 + r)
             for r, (lo, hi) in enumerate(wc)]
    c_wqa = cp(wqkv_hbm.at[:, pl.ds(0, D)], wqkv.at[:, pl.ds(0, D)], 6)
    c_wva = cp(wqkv_hbm.at[:, pl.ds(2 * D, D)], wqkv.at[:, pl.ds(2 * D, D)], 7)
    c_wb = [cp(src.at[:, t], dst.at[pl.ds(1, 64), pl.ds(2 * WP * t, 64), :], 8 + 8 * i + t)
            for i, (src, dst) in enumerate(((wq_hbm, wq), (wk_hbm, wk), (wv_hbm, wv))) for t in range(8)]
    c_late = [cp(wob_hbm.at[:, pl.ds(128 * c, 128)], wob.at[c], 32 + c) for c in range(8)]
    c_late += [cp(woa_hbm.at[:, pl.ds(128 * c, 128)], woa.at[c], 40 + c) for c in range(8)]
    c_late += [
        cp(xb_hbm, xb, 48),
        cp(mem0_hbm, m0v, 49),
    ]
    first = [c_xa[0], c_wka[0], c_wka[1], c_xa[1], c_wka[2], c_xa[2], c_xa[3], c_xa[4], c_wqa, c_wva]
    NF = cfg["NF"]
    for c in first[:NF]:
        c.start()

    qscale = (DHA ** -0.5) * LOG2E

    def kproj(r0, r1, c0, c1):
        if "1" in phases:
            y = jnp.dot(xa[r0:r1, :], wqkv[:, D + c0:D + c1], preferred_element_type=f32)
            yu = _as_u32(y.astype(bf))
            for g in range(c0 // 128, c1 // 128):
                kk[g, r0 // 2:r1 // 2, :] = yu[:, 128 * g - c0:128 * (g + 1) - c0]

    c_xa[0].wait()
    c_wka[0].wait()
    for c in first[NF:]:
        c.start()
    kproj(0, 256, 0, 256)
    c_wka[1].wait()
    kproj(0, 256, 256, 512)
    c_xa[1].wait()
    kproj(256, 512, 0, 512)
    c_wka[2].wait()
    kproj(0, 512, 512, 1024)
    c_xa[2].wait()
    kproj(512, 1024, 0, 1024)
    c_xa[3].wait()
    c_xa[4].wait()
    for c in c_wb:
        c.start()
    kproj(1024, 1536, 0, 1024)
    kproj(1536, 2048, 0, 1024)
    c_wqa.wait()
    c_wva.wait()

    if "1" in phases:
        def a1qv(c, _):
            c0 = pl.multiple_of(c * CC, CC)
            y = lax.dot_general(wqkv[:, pl.ds(c0, CC)], xa[...], TT, preferred_element_type=f32)
            qt[pl.ds(pl.multiple_of(c * (CC // 2), CC // 2), CC // 2), :] = _as_u32((y * qscale).astype(bf))
            y = lax.dot_general(wqkv[:, pl.ds(2 * D + c0, CC)], xa[...], TT, preferred_element_type=f32)
            vt[pl.ds(pl.multiple_of(c * (CC // 2), CC // 2), CC // 2), :] = _as_u32(y.astype(bf))
            cnt[0] = c
            return 0
        lax.fori_loop(0, D // CC, a1qv, 0)

    for c in c_wb:
        c.wait()
    for c in c_late:
        c.start()
    w32 = [w.bitcast(u32) for w in (wq, wk, wv)]

    def relayout(w, b, j, tie):
        lo = tie(w[b + 1, pl.ds(j, 8, stride=WP), :])
        hi = tie(w[b + 1, pl.ds(16 + j, 8, stride=WP), :])
        w[b, 16 * j:16 * j + 8, :] = (lo & jnp.uint32(0xFFFF)) | (hi << 16)
        w[b, 16 * j + 8:16 * j + 16, :] = (lo >> 16) | (hi & jnp.uint32(0xFFFF0000))

    if "2" in phases:
        def mul(x, n):
            return x * n if isinstance(x, int) else pl.multiple_of(x * n, n)

        def qpad(g, j, qi):
            q = _as_bf(qt[pl.ds(mul(4 * g + j, 16), 16), pl.ds(mul(qi, TQ), TQ)])
            parts = []
            if j > 0:
                parts.append(jnp.zeros((32 * j, TQ), bf))
            parts.append(q)
            if j < 3:
                parts.append(jnp.zeros((32 * (3 - j), TQ), bf))
            return jnp.concatenate(parts, axis=0)

        def p1_chunk(g, w, c, sref, m8, tie):
            k = kk[g, pl.ds(c * CK // 2, CK // 2), :]
            k = _as_bf(jnp.concatenate([tie(k[0:8]), k[8:]], axis=0))
            s = jnp.dot(k, w, preferred_element_type=f32)
            sref[pl.ds(c * CK, CK), :] = s
            mm = jnp.max(s.reshape(CK // 8, 8, TQ), axis=0)
            r0 = 8 * cfg["SROW"]
            return (mm if m8 is None else jnp.maximum(m8, mm)), s[r0:r0 + 8]

        def p2_chunk(h, c, sref, m, l8, o):
            s = sref[pl.ds(c * CK, CK), :]
            p = jnp.exp2(s.reshape(CK // 8, 8, TQ) - m[None])
            ll = jnp.sum(p, axis=0)
            v = _as_bf(vt[pl.ds(mul(h, 16), 16), pl.ds(c * CK, CK)])
            oo = jnp.dot(v, p.reshape(CK, TQ).astype(bf), preferred_element_type=f32)
            return (ll if l8 is None else l8 + ll), (oo if o is None else o + oo), oo

        def bmax(m8):
            return jnp.broadcast_to(jnp.max(m8, axis=0, keepdims=True), (8, TQ))

        NI = 8 * NQ
        UL = 4 * NC
        LEAD = NC + SK

        def stream(t_lo, t_hi, ib, state, flag, p1_end, rl):
            mcur, m8, l8, o = state
            never = jnp.full((8, TQ), flag, jnp.int32) < 0
            nev1 = jnp.full((8, 128), flag, jnp.int32) < 0
            gq = {}
            for dlt in range(0, (t_hi + LEAD) // UL + 1):
                gq[dlt] = ((ib + dlt) // NQ, (ib + dlt) % NQ)
            ms = {max(t_lo, 0) // NC: mcur}
            hist = []
            outs = []
            snew = None
            for t in range(t_lo, t_hi):
                sprev, snew = snew, None
                if t + LEAD < p1_end:
                    u1, c1 = divmod(t + LEAD, NC)
                    g2, q2 = gq[u1 // 4]
                    if c1 == 0:
                        m8 = None
                    def ktie(x):
                        if cfg["KLAG"] and len(hist) >= cfg["KLAG"]:
                            oo = hist[-cfg["KLAG"]][3]
                            dep = functools.reduce(jnp.maximum, [oo[24:32, 128 * cc:128 * (cc + 1)] for cc in range(TQ // 128)])
                            x = jnp.where(nev1, _as_u32(dep), x)
                        return x
                    m8, snew = p1_chunk(g2, qpad(g2, u1 % 4, q2), c1, s_refs[u1 % 4], m8, ktie)
                    if c1 == NC - 1:
                        ms[u1] = bmax(m8)
                if t in rl:
                    anchor = _as_u32(m8[:, 0:128])
                    for wi, bi, ji in rl[t]:
                        relayout(w32[wi], bi, ji, lambda x: jnp.where(nev1, anchor, x))
                if t < 0:
                    continue
                u, c = divmod(t, NC)
                g, qi = gq[u // 4]
                mt = ms[u]
                deps = []
                if sprev is not None and cfg["STIE"]:
                    deps.append(sprev)
                if LAG_M and len(hist) >= LAG_M and hist[-LAG_M][0] is not None:
                    deps.append(hist[-LAG_M][0])
                if LAG_L and len(hist) >= LAG_L:
                    deps.append(hist[-LAG_L][1])
                if LAG_O and len(hist) >= LAG_O:
                    oo = hist[-LAG_O][2]
                    deps += [oo[8 * r:8 * r + 8] for r in range(4 - cfg["OROWS"], 4)]
                if deps:
                    mt = jnp.where(never, functools.reduce(jnp.maximum, deps), mt)
                if c == 0:
                    l8 = o = None
                l8, o, oraw = p2_chunk(4 * g + u % 4, c, s_refs[u % 4], mt, l8, o)
                hist.append((m8, l8, o, oraw))
                if c == NC - 1:
                    l = jnp.sum(l8, axis=0, keepdims=True)
                    outs.append(o * (1.0 / l))
                    if u % 4 == 3:
                        og = jnp.concatenate(outs, axis=0).T
                        oa[g, pl.ds(mul(qi, TQ // 2), TQ // 2), :] = _as_u32(og.astype(bf))
                        outs = []
            return ms.get(t_hi // NC), m8, l8, o

        T0 = cfg["T0"]
        BI = cfg["BI"]
        NL = (NI - 1) // BI
        BIG = 1 << 30

        def rl_plan(t_lo, nblk, b0):
            plan = {}
            if "P" in phases:
                for n in range(48 * nblk):
                    plan.setdefault(t_lo + 2 + n // 3, []).append((n % 3, b0 + n // 48, (n // 3) % 16))
            return plan

        state = stream(-LEAD, T0, 0, (None, None, None, None), cnt[0], BIG, {})

        def a2(i, state):
            return stream(T0, T0 + BI * UL, i * BI, state, i, BIG, rl_plan(T0, 2 * BI, 2 * BI * i))
        state = lax.fori_loop(0, NL, a2, state)
        rem = NI - NL * BI
        stream(T0, rem * UL, NL * BI, state, cnt[0], rem * UL, rl_plan(T0, 2 * rem, 2 * BI * NL))

    for c in c_late:
        c.wait()
    wob32 = wob.bitcast(u32)
    woa32 = woa.bitcast(u32)

    def w_head(h):
        return jnp.concatenate([_as_bf(w[0:64, 8 * h:8 * h + 8, :].reshape(512, 128)) for w in w32], axis=1)

    def wo_rows(r0, n):
        return jnp.concatenate([_as_bf(wob32[c, pl.ds(r0 // 2, n // 2), :]) for c in range(8)], axis=1)

    def out_copy(i):
        return cp(outv.at[pl.ds(i * US, US)], out_hbm.at[pl.ds(i * US, US)], 0)

    bscale = (DHB ** -0.5) * LOG2E
    neg = -1e9 * LOG2E
    ri = lax.broadcasted_iota(jnp.int32, (SEG, L), 0)
    ci = lax.broadcasted_iota(jnp.int32, (SEG, L), 1)
    mask = (ri < MEM) | (ci < MEM) | (ci >= SEG) | (ri >= ci)
    G = US * MEM
    ri = lax.broadcasted_iota(jnp.int32, (G, 3 * G), 0)
    ci = lax.broadcasted_iota(jnp.int32, (G, 3 * G), 1)
    own8 = (ci % G) // MEM == ri // MEM
    vis8 = own8 & ((ci < G) | ((ci < 2 * G) & (ci % MEM <= ri % MEM)))
    fill8 = jnp.where(own8, neg, -jnp.inf).astype(f32)
    mult8 = jnp.where(ci >= 2 * G, float((SEG - MEM) // MEM), 1.0).astype(f32)

    def bloop(i, mem):
        first8 = {}
        kv8 = {}
        for u in range(US):
            s = i * US + u
            if "3" in phases:
                o = jnp.concatenate(
                    [_as_bf(oa[g, pl.ds(pl.multiple_of(s * 16, 16), 16), :]) for g in range(8)], axis=1)
                wa = jnp.concatenate([_as_bf(woa32[c]) for c in range(8)], axis=1)
                outv[s, :, 0:D] = jnp.dot(o, wa, preferred_element_type=f32).astype(bf)
            if "B" not in phases:
                continue
            parts = [mem, xb[s, MEM:SEG, :]]
            if u == 0:
                parts.append(xb[pl.ds(i * US, US), 0:MEM, :].reshape(US * MEM, D))
            hs = jnp.concatenate(parts, axis=0)
            qkv = {}
            sc = {}
            sc8 = {}
            os_ = {}

            def proj(h):
                y = jnp.dot(hs, w_head(h), preferred_element_type=f32)
                q = (y[:, 0:128] * bscale).astype(bf)
                if u == 0:
                    first8[h] = (q[SEG:], y[SEG:, 128:384])
                kv = jnp.concatenate([y[0:SEG, 128:384], first8[h][1][MEM * u:MEM * (u + 1)]], axis=0).astype(bf)
                qkv[h] = (q[0:SEG], kv)
                kv8[u, h] = (y[0:MEM, 128:384], y[8:16, 256:384] + y[16:24, 256:384] + y[24:32, 256:384])

            def score(h):
                q, kv = qkv[h]
                t = lax.dot_general(q, kv[:, 0:128], NT, preferred_element_type=f32)
                t = jnp.where(mask, t, neg)
                m = jnp.max(t, axis=1, keepdims=True)
                p = jnp.exp2(t - m)
                l = jnp.sum(p, axis=1, keepdims=True)
                sc[h] = (p * (1.0 / l)).astype(bf)
                if u == US - 1:
                    kv = jnp.concatenate([kv8[v, h][0] for v in range(US)] + [first8[h][1]], axis=0).astype(bf)
                    t = lax.dot_general(first8[h][0], kv[:, 0:128], NT, preferred_element_type=f32)
                    t = jnp.concatenate([t, jnp.zeros((G, G), f32)], axis=1)
                    t = jnp.where(vis8, t, fill8)
                    m = jnp.max(t, axis=1, keepdims=True)
                    p = jnp.exp2(t - m)
                    l = jnp.sum(p * mult8, axis=1, keepdims=True)
                    vx = jnp.concatenate([kv8[v, h][1] for v in range(US)], axis=0).astype(bf)
                    sc8[h] = ((p * (1.0 / l)).astype(bf), jnp.concatenate([kv[:, 128:256], vx], axis=0))

            def pv(h):
                o = jnp.dot(sc[h], qkv[h][1][:, 128:256], preferred_element_type=f32).astype(bf)
                if u == US - 1:
                    o8 = jnp.dot(sc8[h][0], sc8[h][1], preferred_element_type=f32).astype(bf)
                    o = jnp.concatenate([o, o8], axis=0)
                os_[h] = o

            def wo(h0, h1):
                o = jnp.concatenate([os_[h] for h in range(h0, h1)], axis=1)
                return jnp.dot(o, wo_rows(128 * h0, 128 * (h1 - h0)), preferred_element_type=f32)

            acc = None
            for h in range(HB + PVLAG):
                if h < HB:
                    proj(h)
                else:
                    k = h - HB
                    part = wo(3 * k, 3 * k + 3)
                    acc = part if acc is None else acc + part
                if SLAG <= h < HB + SLAG:
                    score(h - SLAG)
                if h >= PVLAG:
                    pv(h - PVLAG)
            acc = acc + wo(3 * PVLAG, HB)
            y = acc.astype(bf)
            mem = y[0:8]
            outv[s, 8:32, D:2 * D] = y[8:32]
            if u == US - 1:
                outv[pl.ds(i * US, US), 0:8, D:2 * D] = acc[32:64].reshape(US, 8, D).astype(bf)
        out_copy(i).start()
        return mem
    lax.fori_loop(0, NSEG // US, bloop, m0v[...])

    for i in range(NSEG // US):
        out_copy(i).wait()
  return kernel


def build(phases="123PB", **kw):
  cfg = dict(CFG)
  cfg.update(kw)

  @functools.partial(jax.jit, static_argnames=("B_seg_len",))
  def fn(A_x, A_wqkv, A_wo, B_x, B_mem0, B_Wq, B_Wk, B_Wv, B_Wo, B_seg_len):
    assert B_seg_len == SEG
    args = (
        A_x.reshape(S, D), A_wqkv, A_wo,
        B_x.reshape(NSEG, SEG, D), B_mem0.reshape(MEM, D),
        B_Wq.reshape(64, 8, 64, 128), B_Wk.reshape(64, 8, 64, 128), B_Wv.reshape(64, 8, 64, 128),
        B_Wo.reshape(HB * DHB, D),
    )
    scratch = [
        pltpu.VMEM((S, D), bf),
        pltpu.VMEM((D, 3 * D), bf),
        pltpu.VMEM((8, D, 128), bf),
        pltpu.VMEM((8, S // 2, 128), u32),
        pltpu.VMEM((D // 2, S), u32),
        pltpu.VMEM((D // 2, S), u32),
        pltpu.VMEM((8, S // 2, 128), u32),
        pltpu.VMEM((S, TQ), f32), pltpu.VMEM((S, TQ), f32), pltpu.VMEM((S, TQ), f32), pltpu.VMEM((S, TQ), f32),
        pltpu.VMEM((NSEG, SEG, D), bf),
        pltpu.VMEM((MEM, D), bf),
        pltpu.VMEM((65, 16 * WP, 128), bf), pltpu.VMEM((65, 16 * WP, 128), bf), pltpu.VMEM((65, 16 * WP, 128), bf),
        pltpu.VMEM((8, HB * DHB, 128), bf),
        pltpu.VMEM((NSEG, SEG, 2 * D), bf),
        pltpu.SMEM((1,), jnp.int32),
        pltpu.SemaphoreType.DMA((53,)),
    ]
    out = pl.pallas_call(
        make_kernel(phases, cfg),
        out_shape=jax.ShapeDtypeStruct((NSEG, SEG, 2 * D), bf),
        in_specs=[pl.BlockSpec(memory_space=pl.ANY)] * 9,
        out_specs=pl.BlockSpec(memory_space=pl.ANY),
        scratch_shapes=scratch,
        compiler_params=pltpu.CompilerParams(vmem_limit_bytes=126 * 1024 * 1024),
    )(*args)
    return out.reshape(1, S, 2 * D)
  return fn


pallas_concat_heads__softmax_full_mha__memory_aug_recurrent_mem_tr__prompt_kernel = build()
```

```python
import functools, math
import jax
import jax.numpy as jnp
from jax import lax
import jax.experimental.pallas as pl
import jax.experimental.pallas.tpu as pltpu

bf = jnp.bfloat16
f32 = jnp.float32
u32 = jnp.uint32
LOG2E = math.log2(math.e)

S = 2048
D = 1024
HA, DHA = 32, 32
HB, DHB = 32, 128
MEM, SEG = 8, 32
NSEG = S // SEG
L = MEM + SEG

TQ = 512
CK = 128
NQ = S // TQ
NC = S // CK
CC = 256
WP = 36
US = 4

NT = (((1,), (1,)), ((), ()))
TT = (((0,), (1,)), ((), ()))

CFG = dict(SK=2, LAG_M=2, LAG_L=1, LAG_O=3, LAG_OE=5, KLAG=2, SLAG=3, PVLAG=6, T0=8, BI=2, NL=14, KIN=128, OSPLIT=0, NOBC=0)


def _as_bf(x):
    return pltpu.bitcast(x, bf)


def _as_u32(x):
    return pltpu.bitcast(x, u32)


def _mul(x, n):
    return x * n if isinstance(x, int) else pl.multiple_of(x * n, n)


def _maxall(xs):
    return functools.reduce(jnp.maximum, xs)


def make_kernel(phases, cfg):
  SK, LAG_M, LAG_L, LAG_O = cfg["SK"], cfg["LAG_M"], cfg["LAG_L"], cfg["LAG_O"]
  SLAG, PVLAG, KLAG = cfg["SLAG"], cfg["PVLAG"], cfg["KLAG"]

  def kernel(xa_hbm, wqkv_hbm, woa_hbm, xb_hbm, mem0_hbm, wq_hbm, wk_hbm, wv_hbm, wob_hbm,
             out_hbm,
             xa, wqkv, woa, kk, qt, vt, oa, s0, s1, s2, s3,
             xb, m0v, wq, wk, wv, wob, outv, cnt, sems):
    s_refs = (s0, s1, s2, s3)

    def cp(src, dst, i):
        return pltpu.make_async_copy(src, dst, sems.at[i])

    xr = [(0, 256), (256, 512), (512, 1024), (1024, 1536), (1536, 2048)]
    wc = [(0, 256), (256, 512), (512, 1024)]
    c_xa = [cp(xa_hbm.at[pl.ds(lo, hi - lo)], xa.at[pl.ds(lo, hi - lo)], 1 + r) for r, (lo, hi) in enumerate(xr)]
    c_wka = [cp(wqkv_hbm.at[:, pl.ds(D + lo, hi - lo)], wqkv.at[:, pl.ds(D + lo, hi - lo)], 6 + r)
             for r, (lo, hi) in enumerate(wc)]
    c_wqa = cp(wqkv_hbm.at[:, pl.ds(0, D)], wqkv.at[:, pl.ds(0, D)], 9)
    c_wva = cp(wqkv_hbm.at[:, pl.ds(2 * D, D)], wqkv.at[:, pl.ds(2 * D, D)], 9)
    c_wb = [cp(src.at[:, t], dst.at[pl.ds(1, 64), pl.ds(2 * WP * t, 64), :], 10)
            for i, (src, dst) in enumerate(((wq_hbm, wq), (wk_hbm, wk), (wv_hbm, wv))) for t in range(8)]
    c_late = [cp(wob_hbm.at[:, pl.ds(128 * c, 128)], wob.at[c], 11) for c in range(8)]
    c_late += [cp(woa_hbm.at[:, pl.ds(128 * c, 128)], woa.at[c], 11) for c in range(8)]
    c_late += [cp(xb_hbm, xb, 11), cp(mem0_hbm, m0v, 11)]
    for c in [c_xa[0], c_wka[0], c_wka[1], c_xa[1], c_wka[2], c_xa[2], c_xa[3], c_xa[4], c_wqa, c_wva]:
        c.start()

    qscale = (DHA ** -0.5) * LOG2E

    def kproj(r0, nr, c0, c1):
        if "1" in phases:
            y = jnp.dot(xa[pl.ds(r0, nr), :], wqkv[:, D + c0:D + c1], preferred_element_type=f32)
            yu = _as_u32(y.astype(bf))
            h0 = r0 // 2 if isinstance(r0, int) else pl.multiple_of(r0 // 2, 8)
            for g in range(c0 // 128, c1 // 128):
                kk[g, pl.ds(h0, nr // 2), :] = yu[:, 128 * g - c0:128 * (g + 1) - c0]

    KIN = cfg["KIN"]
    c_xa[0].wait()
    c_wka[0].wait()
    kproj(0, 256, 0, 256)
    c_wka[1].wait()
    kproj(0, 256, 256, 512)
    c_xa[1].wait()
    kproj(256, 256, 0, 512)
    c_wka[2].wait()
    kproj(0, 512, 512, 1024)
    c_xa[2].wait()
    kproj(512, 512, 0, 1024)
    c_xa[3].wait()
    c_xa[4].wait()
    for c in c_wb:
        c.start()
    if S - 4 * KIN > 1024:
        kproj(1024, S - 4 * KIN - 1024, 0, 1024)
    c_wqa.wait()
    c_wva.wait()

    def a1qv(c, _):
        if KIN:
            kproj(pl.multiple_of(S - 4 * KIN + c * KIN, KIN), KIN, 0, 1024)
        if "1" in phases:
            c0 = pl.multiple_of(c * CC, CC)
            y = lax.dot_general(wqkv[:, pl.ds(c0, CC)], xa[...], TT, preferred_element_type=f32)
            qt[pl.ds(_mul(c, CC // 2), CC // 2), :] = _as_u32((y * qscale).astype(bf))
            y = lax.dot_general(wqkv[:, pl.ds(2 * D + c0, CC)], xa[...], TT, preferred_element_type=f32)
            vt[pl.ds(_mul(c, CC // 2), CC // 2), :] = _as_u32(y.astype(bf))
        cnt[0] = c
        return 0
    lax.fori_loop(0, D // CC, a1qv, 0)

    for c in c_wb:
        c.wait()
    for c in c_late:
        c.start()
    w32 = [w.bitcast(u32) for w in (wq, wk, wv)]

    def relayout(w, b, j, tie):
        lo = tie(w[b + 1, pl.ds(j, 8, stride=WP), :])
        hi = tie(w[b + 1, pl.ds(16 + j, 8, stride=WP), :])
        w[b, 16 * j:16 * j + 8, :] = (lo & jnp.uint32(0xFFFF)) | (hi << 16)
        w[b, 16 * j + 8:16 * j + 16, :] = (lo >> 16) | (hi & jnp.uint32(0xFFFF0000))

    if "2" in phases:
        def qpad(g, j, qi):
            q = _as_bf(qt[pl.ds(_mul(4 * g + j, 16), 16), pl.ds(_mul(qi, TQ), TQ)])
            parts = []
            if j > 0:
                parts.append(jnp.zeros((32 * j, TQ), bf))
            parts.append(q)
            if j < 3:
                parts.append(jnp.zeros((32 * (3 - j), TQ), bf))
            return jnp.concatenate(parts, axis=0)

        def p1_chunk(g, w, c, sref, m8, tie):
            k = kk[g, pl.ds(c * CK // 2, CK // 2), :]
            k = _as_bf(jnp.concatenate([tie(k[0:8]), k[8:]], axis=0))
            s = jnp.dot(k, w, preferred_element_type=f32)
            sref[pl.ds(c * CK, CK), :] = s
            mm = jnp.max(s.reshape(CK // 8, 8, TQ), axis=0)
            return (mm if m8 is None else jnp.maximum(m8, mm)), s[0:8]

        def p2_chunk(h, c, sref, m, l8, o):
            s = sref[pl.ds(c * CK, CK), :]
            p = jnp.exp2(s.reshape(CK // 8, 8, TQ) - m[None])
            for r in range(CK // 8 - 1, -1, -1):
                l8 = p[r] if l8 is None else l8 + p[r]
            v = _as_bf(vt[pl.ds(_mul(h, 16), 16), pl.ds(c * CK, CK)])
            oo = jnp.dot(v, p.reshape(CK, TQ).astype(bf), preferred_element_type=f32)
            return l8, (oo if o is None else o + oo), oo

        def bmax(m8):
            return jnp.broadcast_to(jnp.max(m8, axis=0, keepdims=True), (8, TQ))

        NI = 8 * NQ
        UL = 4 * NC
        LEAD = NC + SK

        def stream(t_lo, t_hi, ib, state, flag, p1_end, rl):
            mcur, m8, l8, o = state
            never = jnp.full((8, TQ), flag, jnp.int32) < 0
            nev1 = jnp.full((8, 128), flag, jnp.int32) < 0
            gq = {}
            for dlt in range(0, (t_hi + LEAD) // UL + 1):
                gq[dlt] = ((ib + dlt) // NQ, (ib + dlt) % NQ)
            ms = {max(t_lo, 0) // NC: mcur}
            hist = []
            outs = []
            snew = None
            for t in range(t_lo, t_hi):
                sprev, snew = snew, None
                if t + LEAD < p1_end:
                    u1, c1 = divmod(t + LEAD, NC)
                    g2, q2 = gq[u1 // 4]
                    if c1 == 0:
                        m8 = None

                    def ktie(x):
                        if len(hist) >= KLAG:
                            oo = hist[-KLAG][3]
                            dep = _maxall([oo[24:32, 128 * cc:128 * (cc + 1)] for cc in range(TQ // 128)])
                            x = jnp.where(nev1, _as_u32(dep), x)
                        return x
                    m8, snew = p1_chunk(g2, qpad(g2, u1 % 4, q2), c1, s_refs[u1 % 4], m8, ktie)
                    if c1 == NC - 1:
                        ms[u1] = bmax(m8)
                if t in rl:
                    anchor = _as_u32(m8[:, 0:128])
                    for wi, bi, ji in rl[t]:
                        relayout(w32[wi], bi, ji, lambda x: jnp.where(nev1, anchor, x))
                if t < 0:
                    continue
                u, c = divmod(t, NC)
                g, qi = gq[u // 4]
                mt = ms[u]
                deps = []
                tail = t + LEAD > p1_end
                if sprev is not None:
                    deps.append(sprev)
                if len(hist) >= LAG_M and not tail:
                    deps.append(hist[-LAG_M][0])
                lag_l = LAG_L + 1 if tail else LAG_L
                if len(hist) >= lag_l:
                    deps.append(hist[-lag_l][1])
                lag_o = cfg["LAG_OE"] if tail else LAG_O
                if len(hist) >= lag_o:
                    oo = hist[-lag_o][2]
                    deps += [oo[8 * r:8 * r + 8] for r in range(4)]
                if deps:
                    mt = jnp.where(never, _maxall(deps), mt)
                if c == 0:
                    l8 = o = None
                l8, o, oraw = p2_chunk(4 * g + u % 4, c, s_refs[u % 4], mt, l8, o)
                hist.append((m8, l8, o, oraw))
                if c == NC - 1:
                    l = jnp.sum(l8, axis=0, keepdims=True)
                    outs.append(o * (1.0 / l))
                    if u % 4 == 3:
                        og = jnp.concatenate(outs, axis=0).T
                        oa[g, pl.ds(_mul(qi, TQ // 2), TQ // 2), :] = _as_u32(og.astype(bf))
                        outs = []
            return ms.get(t_hi // NC), m8, l8, o

        T0 = cfg["T0"]
        BI = cfg["BI"]
        NL = cfg["NL"]
        BIG = 1 << 30

        def rl_plan(ntile, i0):
            plan = {}
            if "P" in phases:
                for n in range(96 * ntile):
                    plan.setdefault(T0 + 2 + n // 3, []).append((n % 3, 2 * i0 + n // 48, (n // 3) % 16))
            return plan

        state = stream(-LEAD, T0, 0, (None, None, None, None), cnt[0], BIG, {})

        def a2(i, state):
            return stream(T0, T0 + BI * UL, i * BI, state, i, BIG, rl_plan(BI, BI * i))

        def a2t(i, state):
            return stream(T0, T0 + UL, i, state, i, BIG, rl_plan(1, i))
        if NL:
            state = lax.fori_loop(0, NL, a2, state)
        state = lax.fori_loop(NL * BI, NI - 1, a2t, state)
        stream(T0, UL, NI - 1, state, cnt[0], UL, rl_plan(1, NI - 1))

    for c in c_late:
        c.wait()
    wob32 = wob.bitcast(u32)
    woa32 = woa.bitcast(u32)

    def w_head(h):
        return jnp.concatenate([_as_bf(w[0:64, 8 * h:8 * h + 8, :].reshape(512, 128)) for w in w32], axis=1)

    def wo_rows(r0, n):
        return jnp.concatenate([_as_bf(wob32[c, pl.ds(r0 // 2, n // 2), :]) for c in range(8)], axis=1)

    def out_piece(*idx):
        return cp(outv.at[idx], out_hbm.at[idx], 0)

    bscale = (DHB ** -0.5) * LOG2E
    neg = -1e9 * LOG2E
    ri = lax.broadcasted_iota(jnp.int32, (SEG, L), 0)
    ci = lax.broadcasted_iota(jnp.int32, (SEG, L), 1)
    mask = (ri < MEM) | (ci < MEM) | (ci >= SEG) | (ri >= ci)
    G = US * MEM
    ri = lax.broadcasted_iota(jnp.int32, (G, 3 * G), 0)
    ci = lax.broadcasted_iota(jnp.int32, (G, 3 * G), 1)
    own8 = (ci % G) // MEM == ri // MEM
    vis8 = own8 & ((ci < G) | ((ci < 2 * G) & (ci % MEM <= ri % MEM)))
    fill8 = jnp.where(own8, neg, -jnp.inf).astype(f32)
    mult8 = jnp.where(ci >= 2 * G, float((SEG - MEM) // MEM), 1.0).astype(f32)

    def bloop(i, mem):
        first8 = {}
        kv8 = {}
        segs = pl.ds(i * US, US)
        for u in range(US):
            s = i * US + u
            if "3" in phases:
                o = jnp.concatenate([_as_bf(oa[g, pl.ds(_mul(s, 16), 16), :]) for g in range(8)], axis=1)
                wa = jnp.concatenate([_as_bf(woa32[c]) for c in range(8)], axis=1)
                outv[s, :, 0:D] = jnp.dot(o, wa, preferred_element_type=f32).astype(bf)
            if u == US - 1 and cfg["OSPLIT"]:
                out_piece(segs, slice(None), pl.ds(0, D)).start()
                out_piece(pl.ds(i * US, US - 1), pl.ds(MEM, SEG - MEM), pl.ds(D, D)).start()
            if "B" not in phases:
                continue
            parts = [mem, xb[s, MEM:SEG, :]]
            if u == 0:
                parts.append(xb[segs, 0:MEM, :].reshape(US * MEM, D))
            hs = jnp.concatenate(parts, axis=0)
            qkv = {}
            sc = {}
            sc8 = {}
            os_ = {}

            def proj(h):
                y = jnp.dot(hs, w_head(h), preferred_element_type=f32)
                q = (y[:, 0:128] * bscale).astype(bf)
                if u == 0:
                    first8[h] = (q[SEG:], y[SEG:, 128:384])
                kv = jnp.concatenate([y[0:SEG, 128:384], first8[h][1][MEM * u:MEM * (u + 1)]], axis=0).astype(bf)
                qkv[h] = (q[0:SEG], kv)
                kv8[u, h] = (y[0:MEM, 128:384], y[8:16, 256:384] + y[16:24, 256:384] + y[24:32, 256:384])

            def score(h):
                q, kv = qkv[h]
                t = lax.dot_general(q, kv[:, 0:128], NT, preferred_element_type=f32)
                t = jnp.where(mask, t, neg)
                m = jnp.max(t, axis=1, keepdims=True)
                p = jnp.exp2(t - m)
                l = jnp.sum(p, axis=1, keepdims=True)
                sc[h] = (p * (1.0 / l)).astype(bf)
                if u == US - 1:
                    kv = jnp.concatenate([kv8[v, h][0] for v in range(US)] + [first8[h][1]], axis=0).astype(bf)
                    t = lax.dot_general(first8[h][0], kv[:, 0:128], NT, preferred_element_type=f32)
                    t = jnp.concatenate([t, jnp.zeros((G, G), f32)], axis=1)
                    t = jnp.where(vis8, t, fill8)
                    m = jnp.max(t, axis=1, keepdims=True)
                    p = jnp.exp2(t - m)
                    l = jnp.sum(p * mult8, axis=1, keepdims=True)
                    vx = jnp.concatenate([kv8[v, h][1] for v in range(US)], axis=0).astype(bf)
                    sc8[h] = ((p * (1.0 / l)).astype(bf), jnp.concatenate([kv[:, 128:256], vx], axis=0))

            def pv(h):
                o = jnp.dot(sc[h], qkv[h][1][:, 128:256], preferred_element_type=f32).astype(bf)
                if u == US - 1:
                    o8 = jnp.dot(sc8[h][0], sc8[h][1], preferred_element_type=f32).astype(bf)
                    o = jnp.concatenate([o, o8], axis=0)
                os_[h] = o

            def wo(h0, h1):
                o = jnp.concatenate([os_[h] for h in range(h0, h1)], axis=1)
                return jnp.dot(o, wo_rows(128 * h0, 128 * (h1 - h0)), preferred_element_type=f32)

            acc = None
            for h in range(HB + PVLAG):
                if h < HB:
                    proj(h)
                else:
                    k = h - HB
                    part = wo(3 * k, 3 * k + 3)
                    acc = part if acc is None else acc + part
                if SLAG <= h < HB + SLAG:
                    score(h - SLAG)
                if h >= PVLAG:
                    pv(h - PVLAG)
            acc = acc + wo(3 * PVLAG, HB)
            y = acc.astype(bf)
            mem = y[0:MEM]
            outv[s, MEM:SEG, D:2 * D] = y[MEM:SEG]
            if u == US - 1:
                outv[segs, 0:MEM, D:2 * D] = acc[SEG:].reshape(US, MEM, D).astype(bf)
        if cfg["OSPLIT"]:
            out_piece(segs, pl.ds(0, MEM), pl.ds(D, D)).start()
            out_piece(pl.ds(i * US + US - 1, 1), pl.ds(MEM, SEG - MEM), pl.ds(D, D)).start()
        else:
            out_piece(segs).start()
        return mem
    lax.fori_loop(0, NSEG // US, bloop, m0v[...])

    cp(outv, out_hbm, 0).wait()
  return kernel


def build(phases="123PB", **kw):
  cfg = dict(CFG)
  cfg.update(kw)

  @functools.partial(jax.jit, static_argnames=("B_seg_len",))
  def fn(A_x, A_wqkv, A_wo, B_x, B_mem0, B_Wq, B_Wk, B_Wv, B_Wo, B_seg_len):
    assert B_seg_len == SEG
    args = (
        A_x.reshape(S, D), A_wqkv, A_wo,
        B_x.reshape(NSEG, SEG, D), B_mem0.reshape(MEM, D),
        B_Wq.reshape(64, 8, 64, 128), B_Wk.reshape(64, 8, 64, 128), B_Wv.reshape(64, 8, 64, 128),
        B_Wo.reshape(HB * DHB, D),
    )
    scratch = [
        pltpu.VMEM((S, D), bf),
        pltpu.VMEM((D, 3 * D), bf),
        pltpu.VMEM((8, D, 128), bf),
        pltpu.VMEM((8, S // 2, 128), u32),
        pltpu.VMEM((D // 2, S), u32),
        pltpu.VMEM((D // 2, S), u32),
        pltpu.VMEM((8, S // 2, 128), u32),
        pltpu.VMEM((S, TQ), f32), pltpu.VMEM((S, TQ), f32), pltpu.VMEM((S, TQ), f32), pltpu.VMEM((S, TQ), f32),
        pltpu.VMEM((NSEG, SEG, D), bf),
        pltpu.VMEM((MEM, D), bf),
        pltpu.VMEM((65, 16 * WP, 128), bf), pltpu.VMEM((65, 16 * WP, 128), bf), pltpu.VMEM((65, 16 * WP, 128), bf),
        pltpu.VMEM((8, HB * DHB, 128), bf),
        pltpu.VMEM((NSEG, SEG, 2 * D), bf),
        pltpu.SMEM((1,), jnp.int32),
        pltpu.SemaphoreType.DMA((12,)),
    ]
    out = pl.pallas_call(
        make_kernel(phases, cfg),
        out_shape=jax.ShapeDtypeStruct((NSEG, SEG, 2 * D), bf),
        in_specs=[pl.BlockSpec(memory_space=pl.ANY)] * 9,
        out_specs=pl.BlockSpec(memory_space=pl.ANY),
        scratch_shapes=scratch,
        compiler_params=pltpu.CompilerParams(vmem_limit_bytes=126 * 1024 * 1024,
                                             disable_bounds_checks=bool(cfg["NOBC"])),
    )(*args)
    return out.reshape(1, S, 2 * D)
  return fn


pallas_concat_heads__softmax_full_mha__memory_aug_recurrent_mem_tr__prompt_kernel = build()
```

```python
import functools
import math

import jax
import jax.numpy as jnp
from jax import lax
import jax.experimental.pallas as pl
import jax.experimental.pallas.tpu as pltpu

bf = jnp.bfloat16
f32 = jnp.float32
u32 = jnp.uint32
LOG2E = math.log2(math.e)

S = 2048
D = 1024
DHA = 32
HB, DHB = 32, 128
MEM, SEG = 8, 32
NSEG = S // SEG
L = MEM + SEG

TQ = 512
CK = 128
NQ = S // TQ
NC = S // CK
NI = 8 * NQ
UL = 4 * NC
LEAD = NC + 2
T0 = 8
BI, NL = 2, 14
CC = 256
KIN = 128
WP = 36
US = 4
SLAG, PVLAG = 3, 6

NT = (((1,), (1,)), ((), ()))
TT = (((0,), (1,)), ((), ()))


def _as_bf(x):
    return pltpu.bitcast(x, bf)


def _as_u32(x):
    return pltpu.bitcast(x, u32)


def _mul(x, n):
    return x * n if isinstance(x, int) else pl.multiple_of(x * n, n)


def _maxall(xs):
    return functools.reduce(jnp.maximum, xs)


def _kernel(xa_hbm, wqkv_hbm, woa_hbm, xb_hbm, mem0_hbm, wq_hbm, wk_hbm, wv_hbm, wob_hbm,
            out_hbm,
            xa, wqkv, woa, kk, qt, vt, oa, s0, s1, s2, s3,
            xb, m0v, wq, wk, wv, wob, outv, cnt, sems):
    s_refs = (s0, s1, s2, s3)
    ws = (wq, wk, wv)

    def cp(src, dst, i):
        return pltpu.make_async_copy(src, dst, sems.at[i])

    xr = [(0, 256), (256, 512), (512, 1024), (1024, 1536), (1536, 2048)]
    wc = [(0, 256), (256, 512), (512, 1024)]
    c_xa = [cp(xa_hbm.at[pl.ds(lo, hi - lo)], xa.at[pl.ds(lo, hi - lo)], 1 + r)
            for r, (lo, hi) in enumerate(xr)]
    c_wka = [cp(wqkv_hbm.at[:, pl.ds(D + lo, hi - lo)], wqkv.at[:, pl.ds(D + lo, hi - lo)], 6 + r)
             for r, (lo, hi) in enumerate(wc)]
    c_wqv = [cp(wqkv_hbm.at[:, pl.ds(c0, D)], wqkv.at[:, pl.ds(c0, D)], 9) for c0 in (0, 2 * D)]
    c_wb = [cp(src.at[:, t], dst.at[pl.ds(1, 64), pl.ds(2 * WP * t, 64), :], 10)
            for src, dst in ((wq_hbm, wq), (wk_hbm, wk), (wv_hbm, wv)) for t in range(8)]
    c_late = [cp(wob_hbm.at[:, pl.ds(128 * c, 128)], wob.at[c], 11) for c in range(8)]
    c_late += [cp(woa_hbm.at[:, pl.ds(128 * c, 128)], woa.at[c], 11) for c in range(8)]
    c_late += [cp(xb_hbm, xb, 11), cp(mem0_hbm, m0v, 11)]
    for c in [c_xa[0], c_wka[0], c_wka[1], c_xa[1], c_wka[2], c_xa[2], c_xa[3], c_xa[4]] + c_wqv:
        c.start()

    for w in ws:
        for t in range(8):
            w[1:65, 2 * WP * t + 64:2 * WP * (t + 1), :] = jnp.zeros((64, 2 * WP - 64, 128), bf)

    qscale = (DHA ** -0.5) * LOG2E

    def kproj(r0, nr, c0, c1):
        y = jnp.dot(xa[pl.ds(r0, nr), :], wqkv[:, D + c0:D + c1], preferred_element_type=f32)
        yu = _as_u32(y.astype(bf))
        h0 = r0 // 2 if isinstance(r0, int) else pl.multiple_of(r0 // 2, 8)
        for g in range(c0 // 128, c1 // 128):
            kk[g, pl.ds(h0, nr // 2), :] = yu[:, 128 * g - c0:128 * (g + 1) - c0]

    c_xa[0].wait()
    c_wka[0].wait()
    kproj(0, 256, 0, 256)
    c_wka[1].wait()
    kproj(0, 256, 256, 512)
    c_xa[1].wait()
    kproj(256, 256, 0, 512)
    c_wka[2].wait()
    kproj(0, 512, 512, 1024)
    c_xa[2].wait()
    kproj(512, 512, 0, 1024)
    c_xa[3].wait()
    c_xa[4].wait()
    for c in c_wb:
        c.start()
    nqv = D // CC
    kproj(1024, S - nqv * KIN - 1024, 0, 1024)
    for c in c_wqv:
        c.wait()

    def a1qv(c, _):
        kproj(pl.multiple_of(S - nqv * KIN + c * KIN, KIN), KIN, 0, 1024)
        c0 = pl.multiple_of(c * CC, CC)
        y = lax.dot_general(wqkv[:, pl.ds(c0, CC)], xa[...], TT, preferred_element_type=f32)
        qt[pl.ds(_mul(c, CC // 2), CC // 2), :] = _as_u32((y * qscale).astype(bf))
        y = lax.dot_general(wqkv[:, pl.ds(2 * D + c0, CC)], xa[...], TT, preferred_element_type=f32)
        vt[pl.ds(_mul(c, CC // 2), CC // 2), :] = _as_u32(y.astype(bf))
        cnt[0] = c
        return 0
    lax.fori_loop(0, nqv, a1qv, 0)

    for c in c_wb:
        c.wait()
    for c in c_late:
        c.start()
    w32 = [w.bitcast(u32) for w in ws]

    def relayout(wi, b, j, tie):
        lo = tie(w32[wi][b + 1, pl.ds(j, 8, stride=WP), :])
        hi = tie(w32[wi][b + 1, pl.ds(16 + j, 8, stride=WP), :])
        ws[wi][b, 32 * j:32 * j + 16, :] = _as_bf((lo & jnp.uint32(0xFFFF)) | (hi << 16))
        ws[wi][b, 32 * j + 16:32 * j + 32, :] = _as_bf((lo >> 16) | (hi & jnp.uint32(0xFFFF0000)))

    def qpad(g, j, qi):
        q = _as_bf(qt[pl.ds(_mul(4 * g + j, 16), 16), pl.ds(_mul(qi, TQ), TQ)])
        parts = []
        if j > 0:
            parts.append(jnp.zeros((DHA * j, TQ), bf))
        parts.append(q)
        if j < 3:
            parts.append(jnp.zeros((DHA * (3 - j), TQ), bf))
        return jnp.concatenate(parts, axis=0)

    def p1_chunk(g, w, c, sref, m8, tie):
        k = kk[g, pl.ds(c * CK // 2, CK // 2), :]
        k = _as_bf(jnp.concatenate([tie(k[0:8]), k[8:]], axis=0))
        s = jnp.dot(k, w, preferred_element_type=f32)
        sref[pl.ds(c * CK, CK), :] = s
        mm = jnp.max(s.reshape(CK // 8, 8, TQ), axis=0)
        return (mm if m8 is None else jnp.maximum(m8, mm)), s[0:8]

    def p2_chunk(h, c, sref, m, l8, o):
        s = sref[pl.ds(c * CK, CK), :]
        p = jnp.exp2(s.reshape(CK // 8, 8, TQ) - m[None])
        for r in range(CK // 8 - 1, -1, -1):
            l8 = p[r] if l8 is None else l8 + p[r]
        v = _as_bf(vt[pl.ds(_mul(h, 16), 16), pl.ds(c * CK, CK)])
        oo = jnp.dot(v, p.reshape(CK, TQ).astype(bf), preferred_element_type=f32)
        return l8, (oo if o is None else o + oo), oo

    def stream(t_lo, t_hi, ib, state, flag, p1_end, rl):
        mcur, m8, l8, o = state
        never = jnp.full((8, TQ), flag, jnp.int32) < 0
        nev1 = jnp.full((8, 128), flag, jnp.int32) < 0
        gq = {d: ((ib + d) // NQ, (ib + d) % NQ) for d in range((t_hi + LEAD) // UL + 1)}
        ms = {max(t_lo, 0) // NC: mcur}
        hist = []
        outs = []
        snew = None
        for t in range(t_lo, t_hi):
            sprev, snew = snew, None
            if t + LEAD < p1_end:
                u1, c1 = divmod(t + LEAD, NC)
                g2, q2 = gq[u1 // 4]
                if c1 == 0:
                    m8 = None

                def ktie(x):
                    if len(hist) >= 2:
                        oo = hist[-2][3]
                        dep = _maxall([oo[24:32, 128 * cc:128 * (cc + 1)] for cc in range(TQ // 128)])
                        x = jnp.where(nev1, _as_u32(dep), x)
                    return x
                m8, snew = p1_chunk(g2, qpad(g2, u1 % 4, q2), c1, s_refs[u1 % 4], m8, ktie)
                if c1 == NC - 1:
                    ms[u1] = jnp.broadcast_to(jnp.max(m8, axis=0, keepdims=True), (8, TQ))
            if t in rl:
                anchor = _as_u32(m8[:, 0:128])
                for wi, bi, ji in rl[t]:
                    relayout(wi, bi, ji, lambda x: jnp.where(nev1, anchor, x))
            if t < 0:
                continue
            u, c = divmod(t, NC)
            g, qi = gq[u // 4]
            tail = t + LEAD > p1_end
            lag_l, lag_o = (2, 5) if tail else (1, 3)
            deps = []
            if sprev is not None:
                deps.append(sprev)
            if len(hist) >= 2 and not tail:
                deps.append(hist[-2][0])
            if len(hist) >= lag_l:
                deps.append(hist[-lag_l][1])
            if len(hist) >= lag_o:
                deps += [hist[-lag_o][2][8 * r:8 * r + 8] for r in range(4)]
            mt = jnp.where(never, _maxall(deps), ms[u]) if deps else ms[u]
            if c == 0:
                l8 = o = None
            l8, o, oraw = p2_chunk(4 * g + u % 4, c, s_refs[u % 4], mt, l8, o)
            hist.append((m8, l8, o, oraw))
            if c == NC - 1:
                l = jnp.sum(l8, axis=0, keepdims=True)
                outs.append(o * (1.0 / l))
                if u % 4 == 3:
                    og = jnp.concatenate(outs, axis=0).T
                    oa[g, pl.ds(_mul(qi, TQ // 2), TQ // 2), :] = _as_u32(og.astype(bf))
                    outs = []
        return ms.get(t_hi // NC), m8, l8, o

    def rl_plan(ntile, i0):
        plan = {}
        for n in range(96 * ntile):
            plan.setdefault(T0 + 2 + n // 3, []).append((n % 3, 2 * i0 + n // 48, (n // 3) % 16))
        return plan

    big = 1 << 30
    state = stream(-LEAD, T0, 0, (None, None, None, None), cnt[0], big, {})
    state = lax.fori_loop(
        0, NL, lambda i, st: stream(T0, T0 + BI * UL, i * BI, st, i, big, rl_plan(BI, BI * i)), state)
    state = lax.fori_loop(
        NL * BI, NI - 1, lambda i, st: stream(T0, T0 + UL, i, st, i, big, rl_plan(1, i)), state)
    stream(T0, UL, NI - 1, state, cnt[0], UL, rl_plan(1, NI - 1))

    for c in c_late:
        c.wait()
    wob32 = wob.bitcast(u32)

    def w_head(h):
        return jnp.concatenate(
            [_as_bf(w[0:64, 8 * h:8 * h + 8, :].reshape(D // 2, 128)) for w in w32], axis=1)

    def wo_rows(r0, n):
        return jnp.concatenate([_as_bf(wob32[c, pl.ds(r0 // 2, n // 2), :]) for c in range(8)], axis=1)

    bscale = (DHB ** -0.5) * LOG2E
    neg = -1e9 * LOG2E
    ri = lax.broadcasted_iota(jnp.int32, (SEG, L), 0)
    ci = lax.broadcasted_iota(jnp.int32, (SEG, L), 1)
    mask = (ri < MEM) | (ci < MEM) | (ci >= SEG) | (ri >= ci)
    G = US * MEM
    ri = lax.broadcasted_iota(jnp.int32, (G, 3 * G), 0)
    ci = lax.broadcasted_iota(jnp.int32, (G, 3 * G), 1)
    own8 = (ci % G) // MEM == ri // MEM
    vis8 = own8 & ((ci < G) | ((ci < 2 * G) & (ci % MEM <= ri % MEM)))
    fill8 = jnp.where(own8, neg, -jnp.inf).astype(f32)
    mult8 = jnp.where(ci >= 2 * G, float((SEG - MEM) // MEM), 1.0).astype(f32)

    def bloop(i, mem):
        first8 = {}
        kv8 = {}
        segs = pl.ds(i * US, US)
        for u in range(US):
            s = i * US + u
            o = jnp.concatenate([_as_bf(oa[g, pl.ds(_mul(s, 16), 16), :]) for g in range(8)], axis=1)
            wa = jnp.concatenate([woa[c] for c in range(8)], axis=1)
            outv[s, :, 0:D] = jnp.dot(o, wa, preferred_element_type=f32).astype(bf)

            parts = [mem, xb[s, MEM:SEG, :]]
            if u == 0:
                parts.append(xb[segs, 0:MEM, :].reshape(G, D))
            hs = jnp.concatenate(parts, axis=0)
            qkv = {}
            sc = {}
            sc8 = {}
            os_ = {}

            def proj(h):
                y = jnp.dot(hs, w_head(h), preferred_element_type=f32)
                q = (y[:, 0:128] * bscale).astype(bf)
                if u == 0:
                    first8[h] = (q[SEG:], y[SEG:, 128:384])
                kv = jnp.concatenate(
                    [y[0:SEG, 128:384], first8[h][1][MEM * u:MEM * (u + 1)]], axis=0).astype(bf)
                qkv[h] = (q[0:SEG], kv)
                kv8[u, h] = (y[0:MEM, 128:384], y[8:16, 256:384] + y[16:24, 256:384] + y[24:32, 256:384])

            def score(h):
                q, kv = qkv[h]
                t = lax.dot_general(q, kv[:, 0:128], NT, preferred_element_type=f32)
                t = jnp.where(mask, t, neg)
                m = jnp.max(t, axis=1, keepdims=True)
                p = jnp.exp2(t - m)
                l = jnp.sum(p, axis=1, keepdims=True)
                sc[h] = (p * (1.0 / l)).astype(bf)
                if u == US - 1:
                    kv = jnp.concatenate(
                        [kv8[v, h][0] for v in range(US)] + [first8[h][1]], axis=0).astype(bf)
                    t = lax.dot_general(first8[h][0], kv[:, 0:128], NT, preferred_element_type=f32)
                    t = jnp.concatenate([t, jnp.zeros((G, G), f32)], axis=1)
                    t = jnp.where(vis8, t, fill8)
                    m = jnp.max(t, axis=1, keepdims=True)
                    p = jnp.exp2(t - m)
                    l = jnp.sum(p * mult8, axis=1, keepdims=True)
                    vx = jnp.concatenate([kv8[v, h][1] for v in range(US)], axis=0).astype(bf)
                    sc8[h] = ((p * (1.0 / l)).astype(bf), jnp.concatenate([kv[:, 128:256], vx], axis=0))

            def pv(h):
                o = jnp.dot(sc[h], qkv[h][1][:, 128:256], preferred_element_type=f32).astype(bf)
                if u == US - 1:
                    o8 = jnp.dot(sc8[h][0], sc8[h][1], preferred_element_type=f32).astype(bf)
                    o = jnp.concatenate([o, o8], axis=0)
                os_[h] = o

            def wo(h0, h1):
                o = jnp.concatenate([os_[h] for h in range(h0, h1)], axis=1)
                return jnp.dot(o, wo_rows(DHB * h0, DHB * (h1 - h0)), preferred_element_type=f32)

            acc = None
            for h in range(HB + PVLAG):
                if h < HB:
                    proj(h)
                else:
                    k = h - HB
                    part = wo(3 * k, 3 * k + 3)
                    acc = part if acc is None else acc + part
                if SLAG <= h < HB + SLAG:
                    score(h - SLAG)
                if h >= PVLAG:
                    pv(h - PVLAG)
            acc = acc + wo(3 * PVLAG, HB)
            y = acc.astype(bf)
            mem = y[0:MEM]
            outv[s, MEM:SEG, D:2 * D] = y[MEM:SEG]
            if u == US - 1:
                outv[segs, 0:MEM, D:2 * D] = acc[SEG:].reshape(US, MEM, D).astype(bf)
        cp(outv.at[segs], out_hbm.at[segs], 0).start()
        return mem
    lax.fori_loop(0, NSEG // US, bloop, m0v[...])

    cp(outv, out_hbm, 0).wait()


@jax.jit
def _run(A_x, A_wqkv, A_wo, B_x, B_mem0, B_Wq, B_Wk, B_Wv, B_Wo):
    args = (
        A_x.reshape(S, D), A_wqkv, A_wo,
        B_x.reshape(NSEG, SEG, D), B_mem0.reshape(MEM, D),
        B_Wq.reshape(64, 8, 64, 128), B_Wk.reshape(64, 8, 64, 128), B_Wv.reshape(64, 8, 64, 128),
        B_Wo.reshape(HB * DHB, D),
    )
    scratch = [
        pltpu.VMEM((S, D), bf),
        pltpu.VMEM((D, 3 * D), bf),
        pltpu.VMEM((8, D, 128), bf),
        pltpu.VMEM((8, S // 2, 128), u32),
        pltpu.VMEM((D // 2, S), u32),
        pltpu.VMEM((D // 2, S), u32),
        pltpu.VMEM((8, S // 2, 128), u32),
        pltpu.VMEM((S, TQ), f32), pltpu.VMEM((S, TQ), f32),
        pltpu.VMEM((S, TQ), f32), pltpu.VMEM((S, TQ), f32),
        pltpu.VMEM((NSEG, SEG, D), bf),
        pltpu.VMEM((MEM, D), bf),
        pltpu.VMEM((65, 16 * WP, 128), bf), pltpu.VMEM((65, 16 * WP, 128), bf),
        pltpu.VMEM((65, 16 * WP, 128), bf),
        pltpu.VMEM((8, HB * DHB, 128), bf),
        pltpu.VMEM((NSEG, SEG, 2 * D), bf),
        pltpu.SMEM((1,), jnp.int32),
        pltpu.SemaphoreType.DMA((12,)),
    ]
    out = pl.pallas_call(
        _kernel,
        out_shape=jax.ShapeDtypeStruct((NSEG, SEG, 2 * D), bf),
        in_specs=[pl.BlockSpec(memory_space=pl.ANY)] * 9,
        out_specs=pl.BlockSpec(memory_space=pl.ANY),
        scratch_shapes=scratch,
        compiler_params=pltpu.CompilerParams(vmem_limit_bytes=120 * 1024 * 1024),
    )(*args)
    return out.reshape(1, S, 2 * D)


def pallas_concat_heads__softmax_full_mha__memory_aug_recurrent_mem_tr__prompt_kernel(
        A_x, A_wqkv, A_wo, B_x, B_mem0, B_Wq, B_Wk, B_Wv, B_Wo, B_seg_len):
    if isinstance(B_seg_len, int):
        assert B_seg_len == SEG, "kernel is specialised for the problem's segment length"
    return _run(A_x, A_wqkv, A_wo, B_x, B_mem0, B_Wq, B_Wk, B_Wv, B_Wo)
```

```python
import functools
import math

import jax
import jax.numpy as jnp
from jax import lax
import jax.experimental.pallas as pl
import jax.experimental.pallas.tpu as pltpu

bf = jnp.bfloat16
f32 = jnp.float32
u32 = jnp.uint32
LOG2E = math.log2(math.e)

S = 2048
D = 1024
DHA = 32
HB, DHB = 32, 128
MEM, SEG = 8, 32
NSEG = S // SEG
L = MEM + SEG

TQ = 512
CK = 128
NQ = S // TQ
NC = S // CK
NI = 8 * NQ
UL = 4 * NC
LEAD = NC + 2
T0 = 8
BI, NL = 2, 14
CC = 256
KIN = 128
WP = 36
US = 4
SLAG, PVLAG = 3, 6

NT = (((1,), (1,)), ((), ()))
TT = (((0,), (1,)), ((), ()))


def _as_bf(x):
    return pltpu.bitcast(x, bf)


def _as_u32(x):
    return pltpu.bitcast(x, u32)


def _mul(x, n):
    return x * n if isinstance(x, int) else pl.multiple_of(x * n, n)


def _maxall(xs):
    return functools.reduce(jnp.maximum, xs)


def _kernel(xa_hbm, wqkv_hbm, woa_hbm, xb_hbm, mem0_hbm, wq_hbm, wk_hbm, wv_hbm, wob_hbm,
            out_hbm,
            xa, wqkv, woa, kk, qt, vt, oa, s0, s1, s2, s3,
            xb, m0v, wq, wk, wv, wob, outv, cnt, sems):
    s_refs = (s0, s1, s2, s3)
    ws = (wq, wk, wv)

    def cp(src, dst, i):
        return pltpu.make_async_copy(src, dst, sems.at[i])

    xr = [(0, 256), (256, 512), (512, 1024), (1024, 1536), (1536, 2048)]
    wc = [(0, 256), (256, 512), (512, 1024)]
    c_xa = [cp(xa_hbm.at[pl.ds(lo, hi - lo)], xa.at[pl.ds(lo, hi - lo)], 1 + r)
            for r, (lo, hi) in enumerate(xr)]
    c_wka = [cp(wqkv_hbm.at[:, pl.ds(D + lo, hi - lo)], wqkv.at[:, pl.ds(D + lo, hi - lo)], 6 + r)
             for r, (lo, hi) in enumerate(wc)]
    c_wqv = [cp(wqkv_hbm.at[:, pl.ds(c0, D)], wqkv.at[:, pl.ds(c0, D)], 9) for c0 in (0, 2 * D)]
    c_wb = [cp(src.at[:, t], dst.at[pl.ds(1, 64), pl.ds(2 * WP * t, 64), :], 10)
            for src, dst in ((wq_hbm, wq), (wk_hbm, wk), (wv_hbm, wv)) for t in range(8)]
    c_late = [cp(wob_hbm.at[:, pl.ds(128 * c, 128)], wob.at[c], 11) for c in range(8)]
    c_late += [cp(woa_hbm.at[:, pl.ds(128 * c, 128)], woa.at[c], 11) for c in range(8)]
    c_late += [cp(xb_hbm, xb, 11), cp(mem0_hbm, m0v, 11)]
    for c in [c_xa[0], c_wka[0], c_wka[1], c_xa[1], c_wka[2], c_xa[2], c_xa[3], c_xa[4]] + c_wqv:
        c.start()

    for w in ws:
        for t in range(8):
            w[1:65, 2 * WP * t + 64:2 * WP * (t + 1), :] = jnp.zeros((64, 2 * WP - 64, 128), bf)

    qscale = (DHA ** -0.5) * LOG2E

    def kproj(r0, nr, c0, c1):
        y = jnp.dot(xa[pl.ds(r0, nr), :], wqkv[:, D + c0:D + c1], preferred_element_type=f32)
        yu = _as_u32(y.astype(bf))
        h0 = r0 // 2 if isinstance(r0, int) else pl.multiple_of(r0 >> 1, 8)
        for g in range(c0 // 128, c1 // 128):
            kk[g, pl.ds(h0, nr // 2), :] = yu[:, 128 * g - c0:128 * (g + 1) - c0]

    c_xa[0].wait()
    c_wka[0].wait()
    kproj(0, 256, 0, 256)
    c_wka[1].wait()
    kproj(0, 256, 256, 512)
    c_xa[1].wait()
    kproj(256, 256, 0, 512)
    c_wka[2].wait()
    kproj(0, 512, 512, 1024)
    c_xa[2].wait()
    kproj(512, 512, 0, 1024)
    c_xa[3].wait()
    c_xa[4].wait()
    for c in c_wb:
        c.start()
    nqv = D // CC
    kproj(1024, S - nqv * KIN - 1024, 0, 1024)
    for c in c_wqv:
        c.wait()

    def a1qv(c, _):
        kproj(pl.multiple_of(S - nqv * KIN + c * KIN, KIN), KIN, 0, 1024)
        c0 = pl.multiple_of(c * CC, CC)
        y = lax.dot_general(wqkv[:, pl.ds(c0, CC)], xa[...], TT, preferred_element_type=f32)
        qt[pl.ds(_mul(c, CC // 2), CC // 2), :] = _as_u32((y * qscale).astype(bf))
        y = lax.dot_general(wqkv[:, pl.ds(2 * D + c0, CC)], xa[...], TT, preferred_element_type=f32)
        vt[pl.ds(_mul(c, CC // 2), CC // 2), :] = _as_u32(y.astype(bf))
        cnt[0] = c
        return 0
    lax.fori_loop(0, nqv, a1qv, 0)

    for c in c_wb:
        c.wait()
    for c in c_late:
        c.start()
    w32 = [w.bitcast(u32) for w in ws]

    def relayout(wi, slots, j, tie):
        b, b1 = slots
        lo = tie(w32[wi][b1, pl.ds(j, 8, stride=WP), :])
        hi = tie(w32[wi][b1, pl.ds(16 + j, 8, stride=WP), :])
        ws[wi][b, 32 * j:32 * j + 16, :] = _as_bf((lo & jnp.uint32(0xFFFF)) | (hi << 16))
        ws[wi][b, 32 * j + 16:32 * j + 32, :] = _as_bf((lo >> 16) | (hi & jnp.uint32(0xFFFF0000)))

    def qpad(j, row, col):
        q = _as_bf(qt[pl.ds(row, 16), pl.ds(col, TQ)])
        parts = []
        if j > 0:
            parts.append(jnp.zeros((DHA * j, TQ), bf))
        parts.append(q)
        if j < 3:
            parts.append(jnp.zeros((DHA * (3 - j), TQ), bf))
        return jnp.concatenate(parts, axis=0)

    def p1_chunk(g, w, c, sref, m8, tie):
        k = kk[g, pl.ds(c * CK // 2, CK // 2), :]
        k = _as_bf(jnp.concatenate([tie(k[0:8]), k[8:]], axis=0))
        s = jnp.dot(k, w, preferred_element_type=f32)
        sref[pl.ds(c * CK, CK), :] = s
        mm = jnp.max(s.reshape(CK // 8, 8, TQ), axis=0)
        return (mm if m8 is None else jnp.maximum(m8, mm)), s[0:8]

    def p2_chunk(h, c, sref, m, l8, o):
        s = sref[pl.ds(c * CK, CK), :]
        p = jnp.exp2(s.reshape(CK // 8, 8, TQ) - m[None]).reshape(CK, TQ)
        for r in range(CK - 8, -1, -8):
            l8 = p[r:r + 8] if l8 is None else l8 + p[r:r + 8]
        v = _as_bf(vt[pl.ds(h, 16), pl.ds(c * CK, CK)])
        oo = jnp.dot(v, p.astype(bf), preferred_element_type=f32)
        return l8, (oo if o is None else o + oo), oo

    def stream(t_lo, t_hi, ib, state, flag, p1_end, rl):
        mcur, m8, l8, o = state
        never = jnp.full((8, TQ), flag, jnp.int32) < 0
        nev1 = jnp.full((8, 128), flag, jnp.int32) < 0
        gq = {d: ((ib + d) >> 2, (ib + d) & 3) for d in range((t_hi + LEAD) // UL + 1)}
        ms = {max(t_lo, 0) // NC: mcur}
        hist = []
        outs = []
        qw = {}
        vrow = {}
        snew = None
        for t in range(t_lo, t_hi):
            sprev, snew = snew, None
            if t + LEAD < p1_end:
                u1, c1 = divmod(t + LEAD, NC)
                g2, q2 = gq[u1 // 4]
                if c1 == 0:
                    m8 = None

                def ktie(x):
                    if len(hist) >= 2:
                        oo = hist[-2][3]
                        dep = _maxall([oo[24:32, 128 * cc:128 * (cc + 1)] for cc in range(TQ // 128)])
                        x = jnp.where(nev1, _as_u32(dep), x)
                    return x
                if u1 not in qw:
                    qw[u1] = (_mul(4 * g2 + u1 % 4, 16), _mul(q2, TQ))
                m8, snew = p1_chunk(g2, qpad(u1 % 4, *qw[u1]), c1, s_refs[u1 % 4], m8, ktie)
                if c1 == NC - 1:
                    ms[u1] = jnp.broadcast_to(jnp.max(m8, axis=0, keepdims=True), (8, TQ))
            if t in rl:
                anchor = _as_u32(m8[:, 0:128])
                for wi, bi, ji in rl[t]:
                    relayout(wi, bi, ji, lambda x: jnp.where(nev1, anchor, x))
            if t < 0:
                continue
            u, c = divmod(t, NC)
            g, qi = gq[u // 4]
            tail = t + LEAD > p1_end
            lag_l, lag_o = (2, 5) if tail else (1, 3)
            deps = []
            if sprev is not None:
                deps.append(sprev)
            if len(hist) >= 2 and not tail:
                deps.append(hist[-2][0])
            if len(hist) >= lag_l:
                deps.append(hist[-lag_l][1])
            if len(hist) >= lag_o:
                deps += [hist[-lag_o][2][8 * r:8 * r + 8] for r in range(4)]
            mt = jnp.where(never, _maxall(deps), ms[u]) if deps else ms[u]
            if c == 0:
                l8 = o = None
            if u not in vrow:
                vrow[u] = _mul(4 * g + u % 4, 16)
            l8, o, oraw = p2_chunk(vrow[u], c, s_refs[u % 4], mt, l8, o)
            hist.append((m8, l8, o, oraw))
            if c == NC - 1:
                l = jnp.sum(l8, axis=0, keepdims=True)
                outs.append(o * (1.0 / l))
                if u % 4 == 3:
                    og = jnp.concatenate(outs, axis=0).T
                    oa[g, pl.ds(_mul(qi, TQ // 2), TQ // 2), :] = _as_u32(og.astype(bf))
                    outs = []
        return ms.get(t_hi // NC), m8, l8, o

    def rl_plan(ntile, i0):
        blk = [2 * i0 + b for b in range(2 * ntile + 1)]
        plan = {}
        for n in range(96 * ntile):
            plan.setdefault(T0 + 2 + n // 3, []).append((n % 3, blk[n // 48:n // 48 + 2], (n // 3) % 16))
        return plan

    big = 1 << 30
    state = stream(-LEAD, T0, 0, (None, None, None, None), cnt[0], big, {})
    state = lax.fori_loop(
        0, NL, lambda i, st: stream(T0, T0 + BI * UL, i * BI, st, i, big, rl_plan(BI, BI * i)), state)
    state = lax.fori_loop(
        NL * BI, NI - 1, lambda i, st: stream(T0, T0 + UL, i, st, i, big, rl_plan(1, i)), state)
    stream(T0, UL, NI - 1, state, cnt[0], UL, rl_plan(1, NI - 1))

    for c in c_late:
        c.wait()
    wob32 = wob.bitcast(u32)

    def w_head(h):
        return jnp.concatenate(
            [_as_bf(w[0:64, 8 * h:8 * h + 8, :].reshape(D // 2, 128)) for w in w32], axis=1)

    def wo_rows(r0, n):
        return jnp.concatenate([_as_bf(wob32[c, pl.ds(r0 // 2, n // 2), :]) for c in range(8)], axis=1)

    bscale = (DHB ** -0.5) * LOG2E
    neg = -1e9 * LOG2E
    ri = lax.broadcasted_iota(jnp.int32, (SEG, L), 0)
    ci = lax.broadcasted_iota(jnp.int32, (SEG, L), 1)
    mask = (ri < MEM) | (ci < MEM) | (ci >= SEG) | (ri >= ci)
    G = US * MEM
    ri = lax.broadcasted_iota(jnp.int32, (G, 3 * G), 0)
    ci = lax.broadcasted_iota(jnp.int32, (G, 3 * G), 1)
    own8 = (ci % G) // MEM == ri // MEM
    vis8 = own8 & ((ci < G) | ((ci < 2 * G) & (ci % MEM <= ri % MEM)))
    fill8 = jnp.where(own8, neg, -jnp.inf).astype(f32)
    mult8 = jnp.where(ci >= 2 * G, float((SEG - MEM) // MEM), 1.0).astype(f32)

    def bloop(i, mem):
        first8 = {}
        kv8 = {}
        segs = pl.ds(i * US, US)
        for u in range(US):
            s = i * US + u
            o = jnp.concatenate([_as_bf(oa[g, pl.ds(_mul(s, 16), 16), :]) for g in range(8)], axis=1)
            wa = jnp.concatenate([woa[c] for c in range(8)], axis=1)
            outv[s, :, 0:D] = jnp.dot(o, wa, preferred_element_type=f32).astype(bf)

            parts = [mem, xb[s, MEM:SEG, :]]
            if u == 0:
                parts.append(xb[segs, 0:MEM, :].reshape(G, D))
            hs = jnp.concatenate(parts, axis=0)
            qkv = {}
            sc = {}
            sc8 = {}
            os_ = {}

            def proj(h):
                y = jnp.dot(hs, w_head(h), preferred_element_type=f32)
                q = (y[:, 0:128] * bscale).astype(bf)
                if u == 0:
                    first8[h] = (q[SEG:], y[SEG:, 128:384])
                kv = jnp.concatenate(
                    [y[0:SEG, 128:384], first8[h][1][MEM * u:MEM * (u + 1)]], axis=0).astype(bf)
                qkv[h] = (q[0:SEG], kv)
                kv8[u, h] = (y[0:MEM, 128:384], y[8:16, 256:384] + y[16:24, 256:384] + y[24:32, 256:384])

            def score(h):
                q, kv = qkv[h]
                t = lax.dot_general(q, kv[:, 0:128], NT, preferred_element_type=f32)
                t = jnp.where(mask, t, neg)
                m = jnp.max(t, axis=1, keepdims=True)
                p = jnp.exp2(t - m)
                l = jnp.sum(p, axis=1, keepdims=True)
                sc[h] = (p * (1.0 / l)).astype(bf)
                if u == US - 1:
                    kv = jnp.concatenate(
                        [kv8[v, h][0] for v in range(US)] + [first8[h][1]], axis=0).astype(bf)
                    t = lax.dot_general(first8[h][0], kv[:, 0:128], NT, preferred_element_type=f32)
                    t = jnp.concatenate([t, jnp.zeros((G, G), f32)], axis=1)
                    t = jnp.where(vis8, t, fill8)
                    m = jnp.max(t, axis=1, keepdims=True)
                    p = jnp.exp2(t - m)
                    l = jnp.sum(p * mult8, axis=1, keepdims=True)
                    vx = jnp.concatenate([kv8[v, h][1] for v in range(US)], axis=0).astype(bf)
                    sc8[h] = ((p * (1.0 / l)).astype(bf), jnp.concatenate([kv[:, 128:256], vx], axis=0))

            def pv(h):
                o = jnp.dot(sc[h], qkv[h][1][:, 128:256], preferred_element_type=f32).astype(bf)
                if u == US - 1:
                    o8 = jnp.dot(sc8[h][0], sc8[h][1], preferred_element_type=f32).astype(bf)
                    o = jnp.concatenate([o, o8], axis=0)
                os_[h] = o

            def wo(h0, h1):
                o = jnp.concatenate([os_[h] for h in range(h0, h1)], axis=1)
                return jnp.dot(o, wo_rows(DHB * h0, DHB * (h1 - h0)), preferred_element_type=f32)

            acc = None
            for h in range(HB + PVLAG):
                if h < HB:
                    proj(h)
                else:
                    k = h - HB
                    part = wo(3 * k, 3 * k + 3)
                    acc = part if acc is None else acc + part
                if SLAG <= h < HB + SLAG:
                    score(h - SLAG)
                if h >= PVLAG:
                    pv(h - PVLAG)
            acc = acc + wo(3 * PVLAG, HB)
            y = acc.astype(bf)
            mem = y[0:MEM]
            outv[s, MEM:SEG, D:2 * D] = y[MEM:SEG]
            if u == US - 1:
                outv[segs, 0:MEM, D:2 * D] = acc[SEG:].reshape(US, MEM, D).astype(bf)
        cp(outv.at[segs], out_hbm.at[segs], 0).start()
        return mem
    lax.fori_loop(0, NSEG // US, bloop, m0v[...])

    cp(outv, out_hbm, 0).wait()


@jax.jit
def _run(A_x, A_wqkv, A_wo, B_x, B_mem0, B_Wq, B_Wk, B_Wv, B_Wo):
    args = (
        A_x.reshape(S, D), A_wqkv, A_wo,
        B_x.reshape(NSEG, SEG, D), B_mem0.reshape(MEM, D),
        B_Wq.reshape(64, 8, 64, 128), B_Wk.reshape(64, 8, 64, 128), B_Wv.reshape(64, 8, 64, 128),
        B_Wo.reshape(HB * DHB, D),
    )
    scratch = [
        pltpu.VMEM((S, D), bf),
        pltpu.VMEM((D, 3 * D), bf),
        pltpu.VMEM((8, D, 128), bf),
        pltpu.VMEM((8, S // 2, 128), u32),
        pltpu.VMEM((D // 2, S), u32),
        pltpu.VMEM((D // 2, S), u32),
        pltpu.VMEM((8, S // 2, 128), u32),
        pltpu.VMEM((S, TQ), f32), pltpu.VMEM((S, TQ), f32),
        pltpu.VMEM((S, TQ), f32), pltpu.VMEM((S, TQ), f32),
        pltpu.VMEM((NSEG, SEG, D), bf),
        pltpu.VMEM((MEM, D), bf),
        pltpu.VMEM((65, 16 * WP, 128), bf), pltpu.VMEM((65, 16 * WP, 128), bf),
        pltpu.VMEM((65, 16 * WP, 128), bf),
        pltpu.VMEM((8, HB * DHB, 128), bf),
        pltpu.VMEM((NSEG, SEG, 2 * D), bf),
        pltpu.SMEM((1,), jnp.int32),
        pltpu.SemaphoreType.DMA((12,)),
    ]
    out = pl.pallas_call(
        _kernel,
        out_shape=jax.ShapeDtypeStruct((NSEG, SEG, 2 * D), bf),
        in_specs=[pl.BlockSpec(memory_space=pl.ANY)] * 9,
        out_specs=pl.BlockSpec(memory_space=pl.ANY),
        scratch_shapes=scratch,
        compiler_params=pltpu.CompilerParams(vmem_limit_bytes=120 * 1024 * 1024),
    )(*args)
    return out.reshape(1, S, 2 * D)


def pallas_concat_heads__softmax_full_mha__memory_aug_recurrent_mem_tr__prompt_kernel(
        A_x, A_wqkv, A_wo, B_x, B_mem0, B_Wq, B_Wk, B_Wv, B_Wo, B_seg_len):
    if isinstance(B_seg_len, int):
        assert B_seg_len == SEG, "kernel is specialised for the problem's segment length"
    return _run(A_x, A_wqkv, A_wo, B_x, B_mem0, B_Wq, B_Wk, B_Wv, B_Wo)
```

```python
import functools
import math

import jax
import jax.numpy as jnp
from jax import lax
import jax.experimental.pallas as pl
import jax.experimental.pallas.tpu as pltpu

bf = jnp.bfloat16
f32 = jnp.float32
u32 = jnp.uint32
LOG2E = math.log2(math.e)

S = 2048
D = 1024
DHA = 32
HB, DHB = 32, 128
MEM, SEG = 8, 32
NSEG = S // SEG
L = MEM + SEG

TQ = 512
CK = 128
NQ = S // TQ
NC = S // CK
NI = 8 * NQ
UL = 4 * NC
LEAD = NC + 2
T0 = 8
BI, NL = 2, 14
CC = 256
KIN = 128
WP = 36
WS = 16 * WP + 64
US = 4
SLAG, PVLAG = 3, 6

NT = (((1,), (1,)), ((), ()))
TT = (((0,), (1,)), ((), ()))


def _as_bf(x):
    return pltpu.bitcast(x, bf)


def _as_u32(x):
    return pltpu.bitcast(x, u32)


def _mul(x, n):
    return x * n if isinstance(x, int) else pl.multiple_of(x * n, n)


def _maxall(xs):
    return functools.reduce(jnp.maximum, xs)


def _kernel(xa_hbm, wqkv_hbm, woa_hbm, xb_hbm, mem0_hbm, wq_hbm, wk_hbm, wv_hbm, wob_hbm,
            out_hbm,
            xa, wqkv, woa, kk, qt, vt, oa, s0, s1, s2, s3,
            xb, m0v, wq, wk, wv, wob, outv, cnt, sems):
    s_refs = (s0, s1, s2, s3)
    ws = (wq, wk, wv)

    def cp(src, dst, i):
        return pltpu.make_async_copy(src, dst, sems.at[i])

    xr = [(0, 256), (256, 512), (512, 1024), (1024, 1536), (1536, 2048)]
    wc = [(0, 256), (256, 512), (512, 1024)]
    c_xa = [cp(xa_hbm.at[pl.ds(lo, hi - lo)], xa.at[pl.ds(lo, hi - lo)], 1 + r)
            for r, (lo, hi) in enumerate(xr)]
    c_wka = [cp(wqkv_hbm.at[:, pl.ds(D + lo, hi - lo)], wqkv.at[:, pl.ds(D + lo, hi - lo)], 6 + r)
             for r, (lo, hi) in enumerate(wc)]
    c_wqv = [cp(wqkv_hbm.at[:, pl.ds(c0, D)], wqkv.at[:, pl.ds(c0, D)], 9) for c0 in (0, 2 * D)]
    c_wb = [cp(src.at[:, t], dst.at[pl.ds(1, 64), pl.ds(2 * WP * t, 64), :], 10)
            for src, dst in ((wq_hbm, wq), (wk_hbm, wk), (wv_hbm, wv)) for t in range(8)]
    c_late = [cp(wob_hbm.at[:, pl.ds(128 * c, 128)], wob.at[c], 11) for c in range(8)]
    c_late += [cp(woa_hbm.at[:, pl.ds(128 * c, 128)], woa.at[c], 11) for c in range(8)]
    c_late += [cp(xb_hbm, xb, 11), cp(mem0_hbm, m0v, 11)]
    for c in [c_xa[0], c_wka[0], c_wka[1], c_xa[1], c_wka[2], c_xa[2], c_xa[3], c_xa[4]] + c_wqv:
        c.start()

    for w in ws:
        for t in range(8):
            w[1:65, 2 * WP * t + 64:2 * WP * (t + 1), :] = jnp.zeros((64, 2 * WP - 64, 128), bf)
        w[1:65, 16 * WP:WS, :] = jnp.zeros((64, WS - 16 * WP, 128), bf)
        w[0] = jnp.zeros((WS, 128), bf)

    qscale = (DHA ** -0.5) * LOG2E

    def kproj(r0, nr, c0, c1):
        y = jnp.dot(xa[pl.ds(r0, nr), :], wqkv[:, D + c0:D + c1], preferred_element_type=f32)
        yu = _as_u32(y.astype(bf))
        h0 = r0 // 2 if isinstance(r0, int) else pl.multiple_of(r0 >> 1, 8)
        for g in range(c0 // 128, c1 // 128):
            kk[g, pl.ds(h0, nr // 2), :] = yu[:, 128 * g - c0:128 * (g + 1) - c0]

    c_xa[0].wait()
    c_wka[0].wait()
    kproj(0, 256, 0, 256)
    c_wka[1].wait()
    kproj(0, 256, 256, 512)
    c_xa[1].wait()
    kproj(256, 256, 0, 512)
    c_wka[2].wait()
    kproj(0, 512, 512, 1024)
    c_xa[2].wait()
    kproj(512, 512, 0, 1024)
    c_xa[3].wait()
    c_xa[4].wait()
    for c in c_wb:
        c.start()
    nqv = D // CC
    kproj(1024, S - nqv * KIN - 1024, 0, 1024)
    for c in c_wqv:
        c.wait()

    def a1qv(c, _):
        kproj(pl.multiple_of(S - nqv * KIN + c * KIN, KIN), KIN, 0, 1024)
        c0 = pl.multiple_of(c * CC, CC)
        y = lax.dot_general(wqkv[:, pl.ds(c0, CC)], xa[...], TT, preferred_element_type=f32)
        qt[pl.ds(_mul(c, CC // 2), CC // 2), :] = _as_u32((y * qscale).astype(bf))
        y = lax.dot_general(wqkv[:, pl.ds(2 * D + c0, CC)], xa[...], TT, preferred_element_type=f32)
        vt[pl.ds(_mul(c, CC // 2), CC // 2), :] = _as_u32(y.astype(bf))
        cnt[0] = c
        return 0
    lax.fori_loop(0, nqv, a1qv, 0)

    for c in c_wb:
        c.wait()
    for c in c_late:
        c.start()
    w32 = [w.bitcast(u32) for w in ws]

    def relayout(wi, slots, j, tie):
        b, b1 = slots
        lo = tie(w32[wi][b1, pl.ds(j, 8, stride=WP), :])
        hi = tie(w32[wi][b1, pl.ds(16 + j, 8, stride=WP), :])
        ws[wi][b, 32 * j:32 * j + 16, :] = _as_bf((lo & jnp.uint32(0xFFFF)) | (hi << 16))
        ws[wi][b, 32 * j + 16:32 * j + 32, :] = _as_bf((lo >> 16) | (hi & jnp.uint32(0xFFFF0000)))

    def qpad(j, row, col):
        q = _as_bf(qt[pl.ds(row, 16), pl.ds(col, TQ)])
        parts = []
        if j > 0:
            parts.append(jnp.zeros((DHA * j, TQ), bf))
        parts.append(q)
        if j < 3:
            parts.append(jnp.zeros((DHA * (3 - j), TQ), bf))
        return jnp.concatenate(parts, axis=0)

    def p1_chunk(g, w, c, sref, m8, tie):
        k = kk[g, pl.ds(c * CK // 2, CK // 2), :]
        k = _as_bf(jnp.concatenate([tie(k[0:8]), k[8:]], axis=0))
        s = jnp.dot(k, w, preferred_element_type=f32)
        sref[pl.ds(c * CK, CK), :] = s
        mm = jnp.max(s.reshape(CK // 8, 8, TQ), axis=0)
        return (mm if m8 is None else jnp.maximum(m8, mm)), s[0:8]

    def p2_chunk(h, c, sref, m, l8, o):
        s = sref[pl.ds(c * CK, CK), :]
        p = jnp.exp2(s.reshape(CK // 8, 8, TQ) - m[None]).reshape(CK, TQ)
        for r in range(CK - 8, -1, -8):
            l8 = p[r:r + 8] if l8 is None else l8 + p[r:r + 8]
        v = _as_bf(vt[pl.ds(h, 16), pl.ds(c * CK, CK)])
        oo = jnp.dot(v, p.astype(bf), preferred_element_type=f32)
        return l8, (oo if o is None else o + oo), oo

    def stream(t_lo, t_hi, ib, state, flag, p1_end, rl):
        mcur, m8, l8, o = state
        never = jnp.full((8, TQ), flag, jnp.int32) < 0
        nev1 = jnp.full((8, 128), flag, jnp.int32) < 0
        gq = {d: ((ib + d) >> 2, (ib + d) & 3) for d in range((t_hi + LEAD) // UL + 1)}
        ms = {max(t_lo, 0) // NC: mcur}
        hist = []
        outs = []
        qw = {}
        vrow = {}
        snew = None
        for t in range(t_lo, t_hi):
            sprev, snew = snew, None
            if t + LEAD < p1_end:
                u1, c1 = divmod(t + LEAD, NC)
                g2, q2 = gq[u1 // 4]
                if c1 == 0:
                    m8 = None

                def ktie(x):
                    if len(hist) >= 2:
                        oo = hist[-2][3]
                        dep = _maxall([oo[24:32, 128 * cc:128 * (cc + 1)] for cc in range(TQ // 128)])
                        x = jnp.where(nev1, _as_u32(dep), x)
                    return x
                if u1 not in qw:
                    qw[u1] = (_mul(4 * g2 + u1 % 4, 16), _mul(q2, TQ))
                m8, snew = p1_chunk(g2, qpad(u1 % 4, *qw[u1]), c1, s_refs[u1 % 4], m8, ktie)
                if c1 == NC - 1:
                    ms[u1] = jnp.broadcast_to(jnp.max(m8, axis=0, keepdims=True), (8, TQ))
            if t in rl:
                anchor = _as_u32(m8[:, 0:128])
                for wi, bi, ji in rl[t]:
                    relayout(wi, bi, ji, lambda x: jnp.where(nev1, anchor, x))
            if t < 0:
                continue
            u, c = divmod(t, NC)
            g, qi = gq[u // 4]
            tail = t + LEAD > p1_end
            lag_l, lag_o = (2, 5) if tail else (1, 3)
            deps = []
            if sprev is not None:
                deps.append(sprev)
            if len(hist) >= 2 and not tail:
                deps.append(hist[-2][0])
            if len(hist) >= lag_l:
                deps.append(hist[-lag_l][1])
            if len(hist) >= lag_o:
                deps += [hist[-lag_o][2][8 * r:8 * r + 8] for r in range(4)]
            mt = jnp.where(never, _maxall(deps), ms[u]) if deps else ms[u]
            if c == 0:
                l8 = o = None
            if u not in vrow:
                vrow[u] = _mul(4 * g + u % 4, 16)
            l8, o, oraw = p2_chunk(vrow[u], c, s_refs[u % 4], mt, l8, o)
            hist.append((m8, l8, o, oraw))
            if c == NC - 1:
                l = jnp.sum(l8, axis=0, keepdims=True)
                outs.append(o * (1.0 / l))
                if u % 4 == 3:
                    og = jnp.concatenate(outs, axis=0).T
                    oa[g, pl.ds(_mul(qi, TQ // 2), TQ // 2), :] = _as_u32(og.astype(bf))
                    outs = []
        return ms.get(t_hi // NC), m8, l8, o

    def rl_plan(ntile, i0):
        blk = [2 * i0 + b for b in range(2 * ntile + 1)]
        plan = {}
        for n in range(96 * ntile):
            plan.setdefault(T0 + 2 + n // 3, []).append((n % 3, blk[n // 48:n // 48 + 2], (n // 3) % 16))
        return plan

    big = 1 << 30
    state = stream(-LEAD, T0, 0, (None, None, None, None), cnt[0], big, {})
    state = lax.fori_loop(
        0, NL, lambda i, st: stream(T0, T0 + BI * UL, i * BI, st, i, big, rl_plan(BI, BI * i)), state)
    state = lax.fori_loop(
        NL * BI, NI - 1, lambda i, st: stream(T0, T0 + UL, i, st, i, big, rl_plan(1, i)), state)
    stream(T0, UL, NI - 1, state, cnt[0], UL, rl_plan(1, NI - 1))

    for c in c_late:
        c.wait()
    wob32 = wob.bitcast(u32)

    def w_head(h):
        return jnp.concatenate(
            [_as_bf(w[0:64, 8 * h:8 * h + 8, :].reshape(D // 2, 128)) for w in w32], axis=1)

    def wo_rows(r0, n):
        return jnp.concatenate([_as_bf(wob32[c, pl.ds(r0 // 2, n // 2), :]) for c in range(8)], axis=1)

    bscale = (DHB ** -0.5) * LOG2E
    neg = -1e9 * LOG2E
    ri = lax.broadcasted_iota(jnp.int32, (SEG, L), 0)
    ci = lax.broadcasted_iota(jnp.int32, (SEG, L), 1)
    mask = (ri < MEM) | (ci < MEM) | (ci >= SEG) | (ri >= ci)
    G = US * MEM
    ri = lax.broadcasted_iota(jnp.int32, (G, 3 * G), 0)
    ci = lax.broadcasted_iota(jnp.int32, (G, 3 * G), 1)
    own8 = (ci % G) // MEM == ri // MEM
    vis8 = own8 & ((ci < G) | ((ci < 2 * G) & (ci % MEM <= ri % MEM)))
    fill8 = jnp.where(own8, neg, -jnp.inf).astype(f32)
    mult8 = jnp.where(ci >= 2 * G, float((SEG - MEM) // MEM), 1.0).astype(f32)

    def bloop(i, mem):
        first8 = {}
        kv8 = {}
        segs = pl.ds(i * US, US)
        for u in range(US):
            s = i * US + u
            o = jnp.concatenate([_as_bf(oa[g, pl.ds(_mul(s, 16), 16), :]) for g in range(8)], axis=1)
            wa = jnp.concatenate([woa[c] for c in range(8)], axis=1)
            outv[s, :, 0:D] = jnp.dot(o, wa, preferred_element_type=f32).astype(bf)

            parts = [mem, xb[s, MEM:SEG, :]]
            if u == 0:
                parts.append(xb[segs, 0:MEM, :].reshape(G, D))
            hs = jnp.concatenate(parts, axis=0)
            qkv = {}
            sc = {}
            sc8 = {}
            os_ = {}

            def proj(h):
                y = jnp.dot(hs, w_head(h), preferred_element_type=f32)
                q = (y[:, 0:128] * bscale).astype(bf)
                if u == 0:
                    first8[h] = (q[SEG:], y[SEG:, 128:384])
                kv = jnp.concatenate(
                    [y[0:SEG, 128:384], first8[h][1][MEM * u:MEM * (u + 1)]], axis=0).astype(bf)
                qkv[h] = (q[0:SEG], kv)
                kv8[u, h] = (y[0:MEM, 128:384], y[8:16, 256:384] + y[16:24, 256:384] + y[24:32, 256:384])

            def score(h):
                q, kv = qkv[h]
                t = lax.dot_general(q, kv[:, 0:128], NT, preferred_element_type=f32)
                t = jnp.where(mask, t, neg)
                m = jnp.max(t, axis=1, keepdims=True)
                p = jnp.exp2(t - m)
                l = jnp.sum(p, axis=1, keepdims=True)
                sc[h] = (p * (1.0 / l)).astype(bf)
                if u == US - 1:
                    kv = jnp.concatenate(
                        [kv8[v, h][0] for v in range(US)] + [first8[h][1]], axis=0).astype(bf)
                    t = lax.dot_general(first8[h][0], kv[:, 0:128], NT, preferred_element_type=f32)
                    t = jnp.concatenate([t, jnp.zeros((G, G), f32)], axis=1)
                    t = jnp.where(vis8, t, fill8)
                    m = jnp.max(t, axis=1, keepdims=True)
                    p = jnp.exp2(t - m)
                    l = jnp.sum(p * mult8, axis=1, keepdims=True)
                    vx = jnp.concatenate([kv8[v, h][1] for v in range(US)], axis=0).astype(bf)
                    sc8[h] = ((p * (1.0 / l)).astype(bf), jnp.concatenate([kv[:, 128:256], vx], axis=0))

            def pv(h):
                o = jnp.dot(sc[h], qkv[h][1][:, 128:256], preferred_element_type=f32).astype(bf)
                if u == US - 1:
                    o8 = jnp.dot(sc8[h][0], sc8[h][1], preferred_element_type=f32).astype(bf)
                    o = jnp.concatenate([o, o8], axis=0)
                os_[h] = o

            def wo(h0, h1):
                o = jnp.concatenate([os_[h] for h in range(h0, h1)], axis=1)
                return jnp.dot(o, wo_rows(DHB * h0, DHB * (h1 - h0)), preferred_element_type=f32)

            acc = None
            for h in range(HB + PVLAG):
                if h < HB:
                    proj(h)
                else:
                    k = h - HB
                    part = wo(3 * k, 3 * k + 3)
                    acc = part if acc is None else acc + part
                if SLAG <= h < HB + SLAG:
                    score(h - SLAG)
                if h >= PVLAG:
                    pv(h - PVLAG)
            acc = acc + wo(3 * PVLAG, HB)
            y = acc.astype(bf)
            mem = y[0:MEM]
            outv[s, MEM:SEG, D:2 * D] = y[MEM:SEG]
            if u == US - 1:
                outv[segs, 0:MEM, D:2 * D] = acc[SEG:].reshape(US, MEM, D).astype(bf)
        cp(outv.at[segs], out_hbm.at[segs], 0).start()
        return mem
    lax.fori_loop(0, NSEG // US, bloop, m0v[...])

    cp(outv, out_hbm, 0).wait()


@jax.jit
def _run(A_x, A_wqkv, A_wo, B_x, B_mem0, B_Wq, B_Wk, B_Wv, B_Wo):
    args = (
        A_x.reshape(S, D), A_wqkv, A_wo,
        B_x.reshape(NSEG, SEG, D), B_mem0.reshape(MEM, D),
        B_Wq.reshape(64, 8, 64, 128), B_Wk.reshape(64, 8, 64, 128), B_Wv.reshape(64, 8, 64, 128),
        B_Wo.reshape(HB * DHB, D),
    )
    scratch = [
        pltpu.VMEM((S, D), bf),
        pltpu.VMEM((D, 3 * D), bf),
        pltpu.VMEM((8, D, 128), bf),
        pltpu.VMEM((8, S // 2, 128), u32),
        pltpu.VMEM((D // 2, S), u32),
        pltpu.VMEM((D // 2, S), u32),
        pltpu.VMEM((8, S // 2, 128), u32),
        pltpu.VMEM((S, TQ), f32), pltpu.VMEM((S, TQ), f32),
        pltpu.VMEM((S, TQ), f32), pltpu.VMEM((S, TQ), f32),
        pltpu.VMEM((NSEG, SEG, D), bf),
        pltpu.VMEM((MEM, D), bf),
        pltpu.VMEM((65, WS, 128), bf), pltpu.VMEM((65, WS, 128), bf),
        pltpu.VMEM((65, WS, 128), bf),
        pltpu.VMEM((8, HB * DHB, 128), bf),
        pltpu.VMEM((NSEG, SEG, 2 * D), bf),
        pltpu.SMEM((1,), jnp.int32),
        pltpu.SemaphoreType.DMA((12,)),
    ]
    out = pl.pallas_call(
        _kernel,
        out_shape=jax.ShapeDtypeStruct((NSEG, SEG, 2 * D), bf),
        in_specs=[pl.BlockSpec(memory_space=pl.ANY)] * 9,
        out_specs=pl.BlockSpec(memory_space=pl.ANY),
        scratch_shapes=scratch,
        compiler_params=pltpu.CompilerParams(vmem_limit_bytes=120 * 1024 * 1024),
    )(*args)
    return out.reshape(1, S, 2 * D)


def pallas_concat_heads__softmax_full_mha__memory_aug_recurrent_mem_tr__prompt_kernel(
        A_x, A_wqkv, A_wo, B_x, B_mem0, B_Wq, B_Wk, B_Wv, B_Wo, B_seg_len):
    if isinstance(B_seg_len, int):
        assert B_seg_len == SEG, "kernel is specialised for the problem's segment length"
    return _run(A_x, A_wqkv, A_wo, B_x, B_mem0, B_Wq, B_Wk, B_Wv, B_Wo)
```
